```python
import os as _os
_os.environ.setdefault("JAX_PLATFORMS", "cpu")
import jax
import jax.numpy as jnp

def _softmax(x, axis=-1):
    return jax.nn.softmax(x, axis=axis)
def _gelu(x):
    return jax.nn.gelu(x, approximate=True)
def _silu(x):
    return jax.nn.silu(x)
def _sigmoid(x):
    return jax.nn.sigmoid(x)
def _layernorm(x, axis=-1, eps=1e-5):
    m = jnp.mean(x, axis=axis, keepdims=True)
    v = jnp.var(x, axis=axis, keepdims=True)
    return (x - m) / jnp.sqrt(v + eps)
def _scatter_add(tgt, idx, src, axis=0):
    return tgt.at[idx].add(src)
def _segment_sum(src, seg, n):
    return jax.ops.segment_sum(src, seg, n)
class _Rng:
    def __init__(self, key):
        self._k = key
    def _next(self):
        self._k, sub = jax.random.split(self._k)
        return sub
    def normal(self, shape):
        return jax.random.normal(self._next(), shape, dtype=jnp.bfloat16)
    def randint(self, lo, hi, shape):
        return jax.random.randint(self._next(), shape, lo, hi, dtype=jnp.int32)
    def uniform(self, shape, lo=0.0, hi=1.0):
        return jax.random.uniform(self._next(), shape, jnp.bfloat16, lo, hi)
    def permutation(self, n):
        return jax.random.permutation(self._next(), n)


kernel_name = 'concat_heads__spectral_gfnet__sliding_block__prompt'

def setup_inputs():
    _rng = _Rng(jax.random.key(int.from_bytes(__import__("os").urandom(4), "little")))
    _w = (lambda a: (lambda t: t.astype(jnp.bfloat16) if jnp.issubdtype(t.dtype, jnp.floating) else t)(jnp.asarray(a)))
    def _A_setup():
        B, S, D = 1, 2048, 640
        Df = D // 2 + 1
        return {
            "x": _w((lambda *s: _rng.normal(s) * 0.05)(B, S, D)),
            "w_r": _w((lambda *s: _rng.normal(s) * 0.4)(S, Df) * 0.02),
            "w_i": _w((lambda *s: _rng.normal(s) * 0.4)(S, Df) * 0.02),
        }
    _A_in = _A_setup()

    def _B_setup():
        B, S, D = 1, 2048, 640
        return {
            "x": _w((lambda *s: _rng.normal(s) * 0.2)(B, S, D)),
            "wqkv": _w((lambda *s: _rng.normal(s) * 0.2)(D, 3 * D)),
            "wo": _w((lambda *s: _rng.normal(s) * 0.05)(D, D)),
        }
    _B_in = _B_setup()

    return {
        "A_x": _A_in["x"],
        "A_w_r": _A_in["w_r"],
        "A_w_i": _A_in["w_i"],
        "B_x": _B_in["x"],
        "B_wqkv": _B_in["wqkv"],
        "B_wo": _B_in["wo"],
    }

def reference(A_x, A_w_r, A_w_i, B_x, B_wqkv, B_wo):
    def _A_ref(x, w_r, w_i):
        B, S, D = x.shape
        X = (lambda x, axes=(-2,-1): jnp.fft.rfft2(x.astype(jnp.float32), axes=axes))(x, axes=(-2, -1))
        W = w_r + 1j * w_i
        X = X * W
        y = (lambda x, s, axes=(-2,-1): jnp.fft.irfft2(x, s=s, axes=axes).astype(jnp.bfloat16))(X, (S, D), axes=(-2, -1))
        return y

    def _B_ref(x, wqkv, wo):
        B, S, D = x.shape
        H = 32; Dh = D // H; W = 256
        qkv = (lambda x, *d: x.transpose(*d))((x @ wqkv).reshape(B, S, 3, H, Dh), 2, 0, 3, 1, 4)
        q, k, v = qkv[0], qkv[1], qkv[2]
        scores = jnp.einsum("bhqd,bhkd->bhqk", q, k) * (Dh ** -0.5)
        idx = jnp.arange(S)
        mask = (idx[:, None] - idx[None, :] >= 0) & (idx[:, None] - idx[None, :] < W)
        scores = jnp.where(mask[None, None], scores, -1e9)
        p = _softmax(scores, axis=-1)
        o = jnp.einsum("bhqk,bhkd->bhqd", p, v)
        return (lambda x, *d: x.transpose(*d))(o, 0, 2, 1, 3).reshape(B, S, D) @ wo

    a = _A_ref(A_x, A_w_r, A_w_i)
    b = _B_ref(B_x, B_wqkv, B_wo)
    return jnp.concatenate([a, b], axis=-1)
```

```python
import numpy as np
import ml_dtypes
import jax
import jax.numpy as jnp
from jax import lax
from jax.experimental import pallas as pl
from jax.experimental.pallas import tpu as pltpu
BFn = ml_dtypes.bfloat16
S, D = 2048, 640
def freq_lanes(c):
    l = np.arange(128)
    return np.where(l < 64, 5*l + c, 5*(l-64) + (5-c))
def d_mats():
    d1 = np.arange(128)[:, None].astype(np.float64)
    out = []
    for c in (1, 2):
        f = freq_lanes(c)[None, :].astype(np.float64)
        sg = np.where(np.arange(128)[None, :] < 64, 1.0, -1.0)
        C = np.cos(2*np.pi*f*d1/D); Sn = -np.sin(2*np.pi*f*d1/D)
        M = np.zeros((256, 256))
        M[:128, :128] = C; M[128:, :128] = -sg*Sn; M[:128, 128:] = Sn; M[128:, 128:] = sg*C
        out.append(M)
    l = np.arange(128)[None, :]
    fre = 5.0*l; fim = 5.0*(l-64)
    M0 = np.where(l <= 64, np.cos(2*np.pi*fre*d1/D), -np.sin(2*np.pi*fim*d1/D))
    MA, MB = out
    IA = MA.T*2.0/D; IB = MB.T*2.0/D
    cf = np.where((l == 0) | (l == 64), 1.0, 2.0)
    I0 = (M0*cf).T / D
    return M0, MA, MB, I0, IA, IB
def s_mats():
    k1 = np.arange(128)[:, None]; n1 = np.arange(128)[None, :]
    F = np.zeros((16, 256, 128)); Hh = np.zeros((16, 256, 128))
    for n2 in range(16):
        ph = 2*np.pi*((k1*(16*n1+n2)) % S)/S
        F[n2, :128] = np.cos(ph); F[n2, 128:] = -np.sin(ph)
        Hh[n2, :128] = np.cos(ph).T/S; Hh[n2, 128:] = np.sin(ph).T/S
    return F, Hh
def a_consts2():
    M0, MA, MB, I0, IA, IB = d_mats()
    dm = np.zeros((6, 256, 256), np.float32)
    dm[0, :128, :128] = M0.T; dm[1] = MA.T; dm[2] = MB.T
    dm[3, :128, :128] = I0; dm[4] = IA; dm[5] = IB
    F, Hh = s_mats()
    FT = np.concatenate([F[:, :128].transpose(0, 2, 1), F[:, 128:].transpose(0, 2, 1)], axis=2)
    return dm.astype(BFn), FT.astype(np.float32).astype(BFn), Hh.astype(np.float32).astype(BFn)

H, DH, WIN = 32, 20, 256
DF = 321
BQ = 128
NB = S // BQ
BF, F32 = jnp.bfloat16, jnp.float32
P = 132
QSCALE = float(DH ** -0.5 * np.log2(np.e))
NEG = -1e30
c1, c2, s1, s2 = (float(np.cos(2*np.pi/5)), float(np.cos(4*np.pi/5)), float(np.sin(2*np.pi/5)), float(np.sin(4*np.pi/5)))
NT = (((1,), (1,)), ((), ()))
def ntdot(a, b): return lax.dot_general(a, b, NT, preferred_element_type=F32)
def dot(a, b): return jnp.dot(a, b, preferred_element_type=F32)

def cmul_const(ar, ai, w):
    wr_, wi_ = round(w.real, 12), round(w.imag, 12)
    if wi_ == 0 and wr_ == 1: return ar, ai
    if wi_ == 0 and wr_ == -1: return -ar, -ai
    if wr_ == 0 and wi_ == 1: return -ai, ar
    if wr_ == 0 and wi_ == -1: return ai, -ar
    if abs(abs(wr_) - abs(wi_)) < 1e-12:
        k = abs(wr_); sr, si = np.sign(wr_), np.sign(wi_)
        if sr > 0 and si > 0: return (ar - ai)*k, (ar + ai)*k
        if sr > 0 and si < 0: return (ar + ai)*k, (ai - ar)*k
        if sr < 0 and si > 0: return (ar + ai)*(-k), (ar - ai)*k
        return (ai - ar)*k, (ar + ai)*(-k)
    return ar*wr_ - ai*wi_, ar*wi_ + ai*wr_

def dft4(x, sign):
    (ar, ai), (br, bi), (cr, ci), (dr, di) = x
    t0r, t0i = ar + cr, ai + ci
    t1r, t1i = ar - cr, ai - ci
    t2r, t2i = br + dr, bi + di
    t3r, t3i = br - dr, bi - di
    if sign < 0:
        x1 = (t1r + t3i, t1i - t3r); x3 = (t1r - t3i, t1i + t3r)
    else:
        x1 = (t1r - t3i, t1i + t3r); x3 = (t1r + t3i, t1i - t3r)
    return [(t0r + t2r, t0i + t2i), x1, (t0r - t2r, t0i - t2i), x3]

def dft16(x, sign):
    cols = []
    for n2 in range(4):
        y = dft4([x[4*n1 + n2] for n1 in range(4)], sign)
        y = [cmul_const(y[k1][0], y[k1][1], np.exp(sign*2j*np.pi*n2*k1/16)) for k1 in range(4)]
        cols.append(y)
    out = [None]*16
    for k1 in range(4):
        z = dft4([cols[n2][k1] for n2 in range(4)], sign)
        for k2 in range(4): out[k1 + 4*k2] = z[k2]
    return out


def kernel(ax_hbm, wr_hbm, wi_hbm, bx_hbm, wqkv_hbm, wo_hbm, ft_hbm, hs_hbm, dm_ref, out_hbm,
           ax_v, wr_v, wi_v, ft_v, hs_v, ts, g_s, wf, outa_v,
           bx_v, wqkv_v, wo_v, kg_s, qT_s, vT_s, s_scr, oT_s, outb_v,
           sem_in, sem_x, sem_outa, sem_outb):
    cp_dm = None
    cp_ax = pltpu.make_async_copy(ax_hbm.at[0], ax_v, sem_in.at[0])
    cp_wr = pltpu.make_async_copy(wr_hbm, wr_v, sem_in.at[1])
    cp_wi = pltpu.make_async_copy(wi_hbm, wi_v, sem_in.at[2])
    cp_ft = pltpu.make_async_copy(ft_hbm, ft_v, sem_in.at[3])
    cp_hs = pltpu.make_async_copy(hs_hbm, hs_v, sem_in.at[4])
    cp_w = pltpu.make_async_copy(wqkv_hbm, wqkv_v, sem_in.at[5])
    cp_wo = pltpu.make_async_copy(wo_hbm, wo_v, sem_in.at[6])
    def cp_x(c):
        return pltpu.make_async_copy(bx_hbm.at[0, pl.ds(c*512, 512), :], bx_v.at[pl.ds(c*512, 512), :], sem_x.at[c])
    cp_ax.start(); cp_ft.start(); cp_wr.start(); cp_wi.start(); cp_hs.start()
    cp_x(0).start(); cp_w.start()
    for c in range(1, 4): cp_x(c).start()
    cp_wo.start()

    cp_ax.wait()
    def st1(b, carry):
        r0 = pl.multiple_of(b * 128, 128)
        xt = [ax_v[pl.ds(r0, 128), 128*t:128*t+128].astype(F32) for t in range(5)]
        b_, c_, d_, e_ = xt[1] + xt[4], xt[2] + xt[3], xt[1] - xt[4], xt[2] - xt[3]
        T = [xt[0] + b_ + c_, xt[0] + c1*b_ + c2*c_, -s1*d_ - s2*e_, xt[0] + c2*b_ + c1*c_, s1*e_ - s2*d_]
        for t in range(5):
            for a in range(8):
                ts[t, pl.ds(8*b + a, 16, stride=P), :] = T[t][16*a:16*a+16]
        return carry
    lax.fori_loop(0, 16, st1, 0)

    cp_wr.wait(); cp_wi.wait()
    def wprep(k2, carry):
        l0 = pl.multiple_of(k2 * 128, 128)
        for a, src in enumerate((wr_v, wi_v)):
            wf[a, k2, 0:320, :] = src[0:320, pl.ds(l0, 128)].astype(F32)
            wf[a, k2, 320:321, :] = src[320:321, pl.ds(l0, 128)].astype(F32)
        return carry
    lax.fori_loop(0, 16, wprep, 0)

    cp_ft.wait()
    def st2(n2, carry):
        base = n2 * P
        T = [ts[t, pl.ds(base, 128), :].astype(BF) for t in range(5)]
        Z0 = ntdot(dm_ref[0, 0:128, 0:128], T[0])
        ZA = ntdot(dm_ref[1], jnp.concatenate(T[1:3], axis=1))
        ZB = ntdot(dm_ref[2], jnp.concatenate(T[3:5], axis=1))
        ZT = jnp.concatenate([Z0, ZA, ZB], axis=0).astype(BF)
        PT = dot(ZT, ft_v[n2])
        g_s[0, n2] = PT[0:128, 0:128]; g_s[1, n2] = PT[0:128, 128:256]
        g_s[2, n2] = PT[128:256, 0:128] - PT[256:384, 128:256]; g_s[3, n2] = PT[128:256, 128:256] + PT[256:384, 0:128]
        g_s[4, n2] = PT[384:512, 0:128] - PT[512:640, 128:256]; g_s[5, n2] = PT[384:512, 128:256] + PT[512:640, 0:128]
        return carry
    lax.fori_loop(0, 16, st2, 0, unroll=16)

    row8 = lax.broadcasted_iota(jnp.int32, (8, 128), 0)
    def filt(g, r0, X, wrow, special=None):
        Y = []
        for k2 in range(16):
            wr = wf[0, k2, pl.ds(wrow, 8, stride=5), :]
            wi = wf[1, k2, pl.ds(wrow, 8, stride=5), :]
            if special is not None:
                wr = jnp.where(special, wf[0, k2, 320:321, :], wr); wi = jnp.where(special, wf[1, k2, 320:321, :], wi)
            xr, xi = X[k2]
            Y.append((xr*wr - xi*wi, xr*wi + xi*wr))
        U = dft16(Y, +1)
        for m2 in range(16):
            g_s[2*g, m2, pl.ds(r0, 8), :] = U[m2][0]
            g_s[2*g+1, m2, pl.ds(r0, 8), :] = U[m2][1]
    def load_fft(g, r0):
        x = [(g_s[2*g, n2, pl.ds(r0, 8), :], g_s[2*g+1, n2, pl.ds(r0, 8), :]) for n2 in range(16)]
        return dft16(x, -1)
    def st3ab(rr, carry):
        for g, (clo, chi) in ((1, (1, 4)), (2, (2, 3))):
            for half, c in ((0, clo), (1, chi)):
                r0 = pl.multiple_of(rr*8 + 64*half, 8)
                filt(g, r0, load_fft(g, r0), 40*rr + c)
        return carry
    lax.fori_loop(0, 8, st3ab, 0)
    def st3g0(rr, first):
        r0 = pl.multiple_of(rr*8, 8) if not first else 0
        r1 = pl.multiple_of(rr*8 + 64, 8) if not first else 64
        Xa = load_fft(0, r0); Xb = load_fft(0, r1)
        Ya, Yb = [], []
        A2, B2 = [], []
        for k2 in range(16):
            ar, ai = Xa[k2]; br, bi = Xb[k2]
            if first:
                keep = row8 == 0
                A2.append((jnp.where(keep, ar, ar - bi), jnp.where(keep, ai, ai + br)))
                B2.append((jnp.where(keep, br, br + ai), jnp.where(keep, bi, bi - ar)))
            else:
                A2.append((ar - bi, ai + br)); B2.append((br + ai, bi - ar))
        filt(0, r0, A2, 40*rr)
        filt(0, r1, B2, 40*rr, special=(row8 == 0) if first else None)
    st3g0(0, True)
    lax.fori_loop(1, 8, lambda rr, c: (st3g0(rr, False), c)[1], 0)

    cp_hs.wait()
    def st4(m2, carry):
        hm = hs_v[m2]
        rhs = jnp.concatenate([g_s[k, m2] for k in range(2, 6)], axis=0).astype(BF)
        Q = ntdot(hm, rhs)
        Qr, Qi = Q[:128], Q[128:]
        z0 = ntdot(hm[:128], g_s[0, m2].astype(BF)) - ntdot(hm[128:], g_s[1, m2].astype(BF))
        zA = jnp.concatenate([Qr[:, 0:128] - Qi[:, 128:256], Qi[:, 0:128] + Qr[:, 128:256]], axis=1).astype(BF)
        zB = jnp.concatenate([Qr[:, 256:384] - Qi[:, 384:512], Qi[:, 256:384] + Qr[:, 384:512]], axis=1).astype(BF)
        V0 = dot(z0.astype(BF), dm_ref[3, 0:128, 0:128])
        U1 = dot(zA, dm_ref[4]); U2 = dot(zB, dm_ref[5])
        U1r, U1i, U2r, U2i = U1[:, :128], U1[:, 128:], U2[:, :128], U2[:, 128:]
        p = V0 + c1*U1r + c2*U2r; q = s1*U1i + s2*U2i
        pp = V0 + c2*U1r + c1*U2r; qq = s2*U1i - s1*U2i
        y = [V0 + U1r + U2r, p - q, pp - qq, pp + qq, p + q]
        for t in range(5):
            ts[t, pl.ds(m2 * P, 128), :] = y[t]
        return carry
    lax.fori_loop(0, 16, st4, 0, unroll=16)

    def st5(b, carry):
        r0 = pl.multiple_of(b * 128, 128)
        for t in range(5):
            z = jnp.concatenate([ts[t, pl.ds(8*b + a, 16, stride=P), :] for a in range(8)], axis=0)
            outa_v[pl.ds(r0, 128), 128*t:128*t+128] = z.astype(BF)
        return carry
    lax.fori_loop(0, 16, st5, 0)
    cp_oa = pltpu.make_async_copy(outa_v, out_hbm.at[0, :, pl.ds(0, D)], sem_outa)
    cp_oa.start()

    lane = lax.broadcasted_iota(jnp.int32, (256, 128), 1)
    padk = jnp.where(lane == 127, NEG, 0.0).astype(BF)
    for j in range(8):
        kg_s[j, 0:256, :] = padk
    vT_s[:, 0:256] = jnp.zeros((D, 256), BF)

    lane128 = lax.broadcasted_iota(jnp.int32, (128, 128), 1)

    def proj(b):
        r0 = pl.multiple_of(b * BQ, BQ)
        x = bx_v[pl.ds(r0, BQ), :]
        qkv = jnp.dot(x, wqkv_v[...], preferred_element_type=F32)
        q = (qkv[:, 0:D] * QSCALE).astype(BF)
        k = qkv[:, D:2*D].astype(BF)
        v = qkv[:, 2*D:3*D].astype(BF)
        for t in range(5):
            qT_s[128*t:128*t+128, pl.ds(r0, BQ)] = q[:, 128*t:128*t+128].T
            vT_s[128*t:128*t+128, pl.ds(r0 + 256, BQ)] = v[:, 128*t:128*t+128].T
        for j in range(8):
            c0 = 80 * j
            t0, off = divmod(c0, 128)
            a = k[:, 128*t0:128*t0+128]
            if off > 0:
                a = pltpu.roll(a, 128 - off, 1)
            if off + 80 > 128:
                bb = pltpu.roll(k[:, 128*t0+128:128*t0+256], 128 - off, 1)
                a = jnp.where(lane128 < 128 - off, a, bb)
            a = jnp.where(lane128 < 80, a, jnp.zeros((), BF))
            kg_s[j, pl.ds(r0 + 256, BQ), :] = a

    row8 = lax.broadcasted_iota(jnp.int32, (8, 128), 0)
    col8 = lax.broadcasted_iota(jnp.int32, (8, 128), 1)
    Dm = row8 - col8
    lo4 = row8 < 4
    r16 = lax.broadcasted_iota(jnp.int32, (16, 128), 0)
    ones_last = jnp.where(r16 == 15, 1.0, 0.0).astype(BF)

    def attn(b):
        q0 = pl.multiple_of(b * BQ, BQ)
        def qk4(j, slot):
            kwin = kg_s[j, pl.ds(q0, 384), :]
            qms = []
            for i in range(4):
                qw = qT_s[pl.ds(80*j + 16*i, 32), pl.ds(q0, 128)]
                r = lax.broadcasted_iota(jnp.int32, (32, 128), 0) + 16*i
                qw = jnp.where((r >= 20*i) & (r < 20*i + 20), qw, jnp.zeros((), BF))
                parts = []
                if i > 0: parts.append(jnp.zeros((16*i, 128), BF))
                parts.append(qw)
                parts.append(jnp.zeros((112 - 16*i - 32, 128), BF))
                parts.append(ones_last)
                qms.append(jnp.concatenate(parts, axis=0))
            qm = jnp.concatenate(qms, axis=1)
            s_scr[slot] = jnp.dot(kwin, qm, preferred_element_type=F32)
        def softmax(slot, i):
            sl = slice(128*i, 128*i + 128)
            cs = [jnp.where(Dm > -8*r, s_scr[slot, 8*r:8*r+8, sl], s_scr[slot, 256+8*r:256+8*r+8, sl]) for r in range(16)]
            c = jnp.concatenate(cs, axis=0)
            s1 = s_scr[slot, 128:256, sl]
            m = jnp.max(jnp.maximum(c, s1), axis=0, keepdims=True)
            pc = jnp.exp2(c - m); p1 = jnp.exp2(s1 - m)
            l = jnp.sum(pc + p1, axis=0, keepdims=True)
            p0 = jnp.concatenate([jnp.where(Dm > -8*r, pc[8*r:8*r+8], 0.0) for r in range(16)], axis=0)
            p2 = pc - p0
            p = jnp.concatenate([p0, p1, p2], axis=0).astype(BF)
            return p, l
        def pv(j, i, p, l):
            vt = vT_s[pl.ds(80*j + 16*i, 32), pl.ds(q0, 384)]
            o = jnp.dot(vt, p, preferred_element_type=F32)
            return o * (1.0 / l)
        qk4(0, 0)
        for j in range(8):
            if j + 1 < 8: qk4(j + 1, (j + 1) % 2)
            outs = []
            for i in range(4):
                p, l = softmax(j % 2, i)
                outs.append(pv(j, i, p, l))
            o0, o1, o2, o3 = outs
            oT = jnp.concatenate([o0[0:16], jnp.where(lo4, o0[16:24], o1[0:8]), o1[8:24], o2[8:24],
                                  jnp.where(lo4, o2[24:32], o3[8:16]), o3[16:32]], axis=0)
            oT_s[80*j:80*j+80, :] = oT.astype(BF)

    def outproj(b):
        r0 = pl.multiple_of(b * BQ, BQ)
        o = jnp.concatenate([oT_s[128*t:128*t+128, :].T for t in range(5)], axis=1)
        y = jnp.dot(o, wo_v[...], preferred_element_type=F32)
        outb_v[pl.ds(r0, BQ), :] = y.astype(BF)
        pltpu.make_async_copy(outb_v.at[pl.ds(r0, BQ), :], out_hbm.at[0, pl.ds(r0, BQ), pl.ds(D, D)], sem_outb).start()

    cp_x(0).wait(); cp_w.wait()
    proj(0)
    cp_wo.wait()
    def body(b, carry):
        @pl.when(((b + 1) % 4 == 0) & (b < NB - 1))
        def _():
            cp_x_dyn = pltpu.make_async_copy(bx_hbm.at[0, pl.ds(0, 512), :], bx_v.at[pl.ds(0, 512), :], sem_x.at[(b + 1) // 4])
            cp_x_dyn.wait()
        attn(b)
        proj(jnp.minimum(b + 1, NB - 1))
        outproj(b)
        return carry
    lax.fori_loop(0, NB, body, 0)
    def wbody(b, carry):
        r0 = pl.multiple_of(b * BQ, BQ)
        pltpu.make_async_copy(outb_v.at[pl.ds(r0, BQ), :], out_hbm.at[0, pl.ds(r0, BQ), pl.ds(D, D)], sem_outb).wait()
        return carry
    lax.fori_loop(0, NB, wbody, 0)
    cp_oa.wait()

_DM, _FT, _HS = a_consts2()

@jax.jit
def pallas_concat_heads__spectral_gfnet__sliding_block__prompt_kernel(A_x, A_w_r, A_w_i, B_x, B_wqkv, B_wo):
    anyspec = pl.BlockSpec(memory_space=pl.ANY)
    vm = pl.BlockSpec(memory_space=pltpu.VMEM)
    V = pltpu.VMEM
    return pl.pallas_call(
        kernel,
        out_shape=jax.ShapeDtypeStruct((1, S, 2*D), BF),
        in_specs=[anyspec]*8 + [vm], out_specs=anyspec,
        scratch_shapes=[
            V((S, D), BF), V((DF, S), BF), V((DF, S), BF), V((16, 128, 256), BF), V((16, 256, 128), BF),
            V((5, 16*P, 128), F32), V((6, 16, 128, 128), F32), V((2, 16, 328, 128), F32), V((S, D), BF),
            V((S, D), BF), V((D, 3*D), BF), V((D, D), BF),
            V((8, S + 256, 128), BF), V((D, S), BF), V((D, S + 256), BF),
            V((2, 384, 512), F32), V((D, BQ), BF), V((S, D), BF),
            pltpu.SemaphoreType.DMA((7,)), pltpu.SemaphoreType.DMA((4,)), pltpu.SemaphoreType.DMA(()), pltpu.SemaphoreType.DMA(()),
        ],
        compiler_params=pltpu.CompilerParams(vmem_limit_bytes=110*2**20),
        name="gfnet_swa",
    )(A_x, A_w_r.T, A_w_i.T, B_x, B_wqkv, B_wo, jnp.asarray(_FT), jnp.asarray(_HS), jnp.asarray(_DM))
```

```python
import contextlib
def scope(n): return contextlib.nullcontext()
import numpy as np
import ml_dtypes
import jax
import jax.numpy as jnp
from jax import lax
from jax.experimental import pallas as pl
from jax.experimental.pallas import tpu as pltpu
BFn = ml_dtypes.bfloat16

S, D, H, DH = 2048, 640, 32, 20
DF = 321
BQ = 128
NB = S // BQ
BF, F32, U32 = jnp.bfloat16, jnp.float32, jnp.uint32
QSCALE = float(DH ** -0.5 * np.log2(np.e))
NEG = -1e30
P = 132
c1, c2, s1, s2 = (float(np.cos(2*np.pi/5)), float(np.cos(4*np.pi/5)), float(np.sin(2*np.pi/5)), float(np.sin(4*np.pi/5)))
E = lambda k, d: d
HP = E("HP", 2); LA = E("LA", 1); LB = E("LB", 3)
NQ = 128 // HP; NP = NQ // 16; NMID = (256 - NQ) // 16; NGRP = 2*NP + NMID
NT = (((1,), (1,)), ((), ()))
def freq_lanes(c):
    l = np.arange(128)
    return np.where(l < 64, 5*l + c, 5*(l-64) + (5-c))
def d_mats():
    d1 = np.arange(128)[:, None].astype(np.float64)
    out = []
    for c in (1, 2):
        f = freq_lanes(c)[None, :].astype(np.float64)
        sg = np.where(np.arange(128)[None, :] < 64, 1.0, -1.0)
        C = np.cos(2*np.pi*f*d1/D); Sn = -np.sin(2*np.pi*f*d1/D)
        M = np.zeros((256, 256))
        M[:128, :128] = C; M[128:, :128] = -sg*Sn; M[:128, 128:] = Sn; M[128:, 128:] = sg*C
        out.append(M)
    l = np.arange(128)[None, :]
    fre = 5.0*l; fim = 5.0*(l-64)
    M0 = np.where(l <= 64, np.cos(2*np.pi*fre*d1/D), -np.sin(2*np.pi*fim*d1/D))
    MA, MB = out
    IA = MA.T*2.0/D; IB = MB.T*2.0/D
    cf = np.where((l == 0) | (l == 64), 1.0, 2.0)
    I0 = (M0*cf).T / D
    return M0, MA, MB, I0, IA, IB
def s_mats():
    k1 = np.arange(128)[:, None]; n1 = np.arange(128)[None, :]
    F = np.zeros((16, 256, 128)); Hh = np.zeros((16, 256, 128))
    for n2 in range(16):
        ph = 2*np.pi*((k1*(16*n1+n2)) % S)/S
        F[n2, :128] = np.cos(ph); F[n2, 128:] = -np.sin(ph)
        Hh[n2, :128] = np.cos(ph).T/S; Hh[n2, 128:] = np.sin(ph).T/S
    return F, Hh
def a_consts2():
    M0, MA, MB, I0, IA, IB = d_mats()
    dm = np.zeros((6, 256, 256), np.float32)
    dm[0, :128, :128] = M0.T; dm[1] = MA.T; dm[2] = MB.T
    dm[3, :128, :128] = I0; dm[4] = IA; dm[5] = IB
    F, Hh = s_mats()
    FT = np.concatenate([F[:, :128].transpose(0, 2, 1), F[:, 128:].transpose(0, 2, 1)], axis=2)
    return dm.astype(BFn), FT.astype(np.float32).astype(BFn), Hh.astype(np.float32).astype(BFn)

def a_consts3():
    dm, FT, HS = a_consts2()
    perm = np.arange(128).reshape(8, 2, 8).transpose(0, 2, 1).reshape(128)
    dm = dm.copy()
    dm[3, :128] = dm[3, :128][perm]
    for k in (4, 5):
        dm[k, :128] = dm[k, :128][perm]
        dm[k, 128:] = dm[k, 128:][perm]
    return dm, FT, HS

def cmul_const(ar, ai, w):
    wr_, wi_ = round(w.real, 12), round(w.imag, 12)
    if wi_ == 0 and wr_ == 1: return ar, ai
    if wi_ == 0 and wr_ == -1: return -ar, -ai
    if wr_ == 0 and wi_ == 1: return -ai, ar
    if wr_ == 0 and wi_ == -1: return ai, -ar
    if abs(abs(wr_) - abs(wi_)) < 1e-12:
        k = abs(wr_); sr, si = np.sign(wr_), np.sign(wi_)
        if sr > 0 and si > 0: return (ar - ai)*k, (ar + ai)*k
        if sr > 0 and si < 0: return (ar + ai)*k, (ai - ar)*k
        if sr < 0 and si > 0: return (ar + ai)*(-k), (ar - ai)*k
        return (ai - ar)*k, (ar + ai)*(-k)
    return ar*wr_ - ai*wi_, ar*wi_ + ai*wr_

def dft4(x, sign):
    (ar, ai), (br, bi), (cr, ci), (dr, di) = x
    t0r, t0i = ar + cr, ai + ci
    t1r, t1i = ar - cr, ai - ci
    t2r, t2i = br + dr, bi + di
    t3r, t3i = br - dr, bi - di
    if sign < 0:
        x1 = (t1r + t3i, t1i - t3r); x3 = (t1r - t3i, t1i + t3r)
    else:
        x1 = (t1r - t3i, t1i + t3r); x3 = (t1r + t3i, t1i - t3r)
    return [(t0r + t2r, t0i + t2i), x1, (t0r - t2r, t0i - t2i), x3]

def dft16(x, sign):
    cols = []
    for n2 in range(4):
        y = dft4([x[4*n1 + n2] for n1 in range(4)], sign)
        y = [cmul_const(y[k1][0], y[k1][1], np.exp(sign*2j*np.pi*n2*k1/16)) for k1 in range(4)]
        cols.append(y)
    out = [None]*16
    for k1 in range(4):
        z = dft4([cols[n2][k1] for n2 in range(4)], sign)
        for k2 in range(4): out[k1 + 4*k2] = z[k2]
    return out


def ntdot(a, b): return lax.dot_general(a, b, NT, preferred_element_type=F32)
def dot(a, b): return jnp.dot(a, b, preferred_element_type=F32)
def bc(x): return pltpu.bitcast(x, BF)
def pk2(a, b): return pltpu.pack_elementwise([a, b], packed_dtype=BF)
def tree(xs, f):
    xs = list(xs)
    while len(xs) > 1:
        xs = [f(xs[k], xs[k+1]) if k + 1 < len(xs) else xs[k] for k in range(0, len(xs), 2)]
    return xs[0]
def split_pieces(groups, firsts, lasts, flip):
    units = [[f, l] for f, l in zip(firsts, lasts) if f in groups and l in groups]
    paired = {g for u in units for g in u}
    singles = [g for g in groups if g not in paired]
    n = len(groups)
    sizes = [n // 4] * 4
    order = [2, 3, 0, 1] if flip else [0, 1, 2, 3]
    for k in range(n - sum(sizes)): sizes[order[k]] += 1
    pcs = [[] for _ in range(4)]
    k = 0
    for u in units:
        tries = 0
        while len(pcs[k]) + 2 > sizes[k] and tries < 4: k = (k + 1) % 4; tries += 1
        if tries == 4: singles += u; continue
        pcs[k] += u; k = (k + 1) % 4
    for k in range(4):
        while len(pcs[k]) < sizes[k]: pcs[k].append(singles.pop(0))
    assert not singles
    return [p for p in pcs if p]

def kernel(ax_hbm, wr_hbm, wi_hbm, bx_hbm, wqkv_hbm, wo_hbm, ft_hbm, hs_hbm, dm_hbm, out_hbm,
           ax_v, wr_v, wi_v, ft_v, hs_v, dm_v, ts, g_s, u_s, wf, outa_v,
           bx_v, wqkv_v, wo_v, kg_s, qT_s, vT_s, oT_s, outb_v, kt_s, ol_s,
           sem_w, sem_x, sem_a, sem_outa, sem_outb):
    WORDER = [5, 6, 7, 8, 9, 0, 1, 2, 3, 4, 10, 11, 12, 13, 14]
    def cp_w(n): return pltpu.make_async_copy(wqkv_hbm.at[:, pl.ds(128*n, 128)], wqkv_v.at[:, pl.ds(128*n, 128)], sem_w.at[n])
    XCH = [(0, 256), (256, 512), (512, 1024), (1024, 1536), (1536, 2048)]
    def cp_x(c):
        lo, hi = XCH[c]
        return pltpu.make_async_copy(bx_hbm.at[0, pl.ds(lo, hi - lo), :], bx_v.at[pl.ds(lo, hi - lo), :], sem_x.at[c])
    ACH = [(0, 1024), (1024, 2048)]
    def cp_a(c):
        lo, hi = ACH[c]
        return pltpu.make_async_copy(ax_hbm.at[0, pl.ds(lo, hi - lo), :], ax_v.at[pl.ds(lo, hi - lo), :], sem_a.at[c])
    cp_wr = pltpu.make_async_copy(wr_hbm, wr_v, sem_a.at[2])
    cp_wi = pltpu.make_async_copy(wi_hbm, wi_v, sem_a.at[3])
    cp_ft = pltpu.make_async_copy(ft_hbm, ft_v, sem_a.at[4])
    cp_hs = pltpu.make_async_copy(hs_hbm, hs_v, sem_a.at[5])
    cp_dm = pltpu.make_async_copy(dm_hbm, dm_v, sem_a.at[6])
    cp_wo = pltpu.make_async_copy(wo_hbm, wo_v, sem_w.at[15])
    cp_x(0).start()
    for n in WORDER[:10]: cp_w(n).start()

    row8 = lax.broadcasted_iota(jnp.int32, (8, 128), 0)
    col8 = lax.broadcasted_iota(jnp.int32, (8, 128), 1)
    col64 = lax.broadcasted_iota(jnp.int32, (64, 128), 1)
    DQ = row8 - (col8 & (NQ - 1))
    lo4 = row8 < 4
    part = col8 >> int(np.log2(NQ)) if HP > 1 else col8 * 0
    bits = [((part >> k) & 1) == 1 for k in range(int(np.log2(HP)))]
    zero_u = jnp.zeros((8, 128), U32)

    def proj_items(b):
        r0 = b * BQ; u0 = b * 64
        def mm(n): return dot(bx_v[pl.ds(r0, BQ), :], wqkv_v[:, 128*n:128*n+128])
        def qtile(t):
            def f():
                q = (mm(t) * QSCALE).astype(BF)
                qT_s[64*t:64*t+64, pl.ds(r0, BQ)] = pltpu.bitcast(q.T, U32)
            return f
        def vtile(t):
            def f():
                v = mm(10 + t)
                w = pk2(jnp.concatenate([v[16*g:16*g+8] for g in range(8)], axis=0),
                        jnp.concatenate([v[16*g+8:16*g+16] for g in range(8)], axis=0))
                vT_s[128*t:128*t+128, pl.ds(r0, BQ)] = bc(w).T.astype(F32)
            return f
        def ktile(t):
            def f(): kt_s[b % 2, t] = pltpu.bitcast(mm(5 + t).astype(BF), U32)
            return f
        def kgrp(j):
            def f():
                t0, off = divmod(80 * j, 128)
                a = kt_s[b % 2, t0]
                if off > 0: a = pltpu.roll(a, 128 - off, 1)
                if off + 80 > 128:
                    a = jnp.where(col64 < 128 - off, a, pltpu.roll(kt_s[b % 2, t0 + 1], 128 - off, 1))
                kg_s[j, pl.ds(u0, 64), :] = jnp.where(col64 < 80, a, U32(0))
            return f
        by_tile = {5: [ktile(0), kgrp(0)], 6: [ktile(1), kgrp(1), kgrp(2)], 7: [ktile(2), kgrp(3)], 8: [ktile(3), kgrp(4), kgrp(5)], 9: [ktile(4), kgrp(6), kgrp(7)]}
        for t in range(5):
            by_tile[t] = [qtile(t)]; by_tile[10 + t] = [vtile(t)]
        return by_tile

    def outproj_items(b):
        r0 = b * BQ
        def tr(t):
            def f(): ol_s[:, 128*t:128*t+128] = pltpu.bitcast(oT_s[b % 2, 128*t:128*t+128, :].astype(BF).T, U32)
            return f
        def mm(n):
            def f(): outb_v[pl.ds(r0, BQ), 128*n:128*n+128] = dot(bc(ol_s[...]), wo_v[:, 128*n:128*n+128]).astype(BF)
            return f
        def dma():
            out_b(b).start()
        return [tr(t) for t in range(5)] + [mm(n) for n in range(5)] + [dma]
    def out_b(b):
        return pltpu.make_async_copy(outb_v.at[pl.ds(b*BQ, BQ), :], out_hbm.at[0, pl.ds(b*BQ, BQ), pl.ds(D, D)], sem_outb)
    def out_a(b):
        return pltpu.make_async_copy(outa_v.at[pl.ds(b*BQ, BQ), :], out_hbm.at[0, pl.ds(b*BQ, BQ), pl.ds(0, D)], sem_outa)

    def attn(b, extras):
        q0 = b * 128
        def make_R(j, heads):
            R = {}
            for ii, i in enumerate(heads):
                lo, hi = 10*i, 10*i + 10
                for t in range(lo//8, (hi-1)//8 + 1):
                    q = qT_s[pl.ds(40*j + 8*t, 8), pl.ds(q0, 128)]
                    if ii > 0: q = pltpu.roll(q, NQ*ii, 1)
                    rlo, rhi = max(lo - 8*t, 0), min(hi - 8*t, 8)
                    R.setdefault(t, []).append((ii, q, rlo, rhi))
            return R
        def make_qm(R, a):
            out = []
            for t in range(5):
                if t not in R: out.append(zero_u); continue
                v = zero_u
                for (ii, q, rlo, rhi) in R[t]:
                    full = (rlo == 0 and rhi == 8)
                    msk = None if full else ((row8 >= rlo) & (row8 < rhi))
                    if HP > 1:
                        pm = part == (ii + a) % HP
                        msk = pm if msk is None else (msk & pm)
                    v = q if msk is None else jnp.where(msk, q, v)
                out.append(v)
            return bc(jnp.concatenate(out, axis=0))
        def key0(a): return q0 - 256 + NQ * a
        def valid(a):
            return [g for g in range(NGRP) if key0(a) + 16*g >= 0]
        def qk_tile(j, a, R):
            qm = make_qm(R, a)
            base = (key0(a)) // 2
            def rows(ids): return bc(jnp.concatenate([kg_s[j, pl.ds(base + 8*g, 8), :] for g in ids], axis=0))[:, 0:80]
            vals = {}
            for ids in split_pieces(valid(a), list(range(NP)), list(range(NP + NMID, NGRP)), a % 2):
                s = dot(rows(ids), qm)
                for n, g in enumerate(ids):
                    vals[g] = (s[16*n:16*n+8], s[16*n+8:16*n+16])
            cs = []
            for r in range(2*NP):
                g, hh = divmod(r, 2)
                fst = vals[g][hh] if g in vals else NEG
                cs.append(jnp.where(DQ > -8*r, fst, vals[NP + NMID + g][hh]))
            mid = {g: vals[g] for g in range(NP, NP + NMID) if g in vals}
            return cs, mid, [g in vals for g in range(NP)]
        def sm_tile(cs, mid, has_first):
            allv = cs + [x for g in mid for x in mid[g]]
            m = jnp.max(tree(allv, jnp.maximum), axis=0, keepdims=True)
            pc = [jnp.exp2(c - m) for c in cs]
            Pg = {}
            for g in range(NP):
                if has_first[g]:
                    p0 = [jnp.where(DQ > -8*(2*g + hh), pc[2*g + hh], 0.0) for hh in range(2)]
                    Pg[g] = pk2(p0[0], p0[1])
                    Pg[NP + NMID + g] = pk2(pc[2*g] - p0[0], pc[2*g + 1] - p0[1])
                else:
                    Pg[NP + NMID + g] = pk2(pc[2*g], pc[2*g + 1])
            for g in mid:
                Pg[g] = pk2(jnp.exp2(mid[g][0] - m), jnp.exp2(mid[g][1] - m))
            return Pg
        kt_lo = max(0, (256 - q0) // 128)
        def merge(Ps):
            out = [[] for _ in range(HP)]
            for gam in range(8 * kt_lo, 24):
                s = [Ps[a].get(gam - NP*a) if 0 <= gam - NP*a < NGRP else None for a in range(HP)]
                def sel(mask, x, y):
                    if x is None and y is None: return None
                    return jnp.where(mask, zero_u if x is None else x, zero_u if y is None else y)
                w = s
                for k, bit in enumerate(bits):
                    w = [sel(bit, w[(n + (1 << k)) % HP], w[n]) for n in range(HP)]
                if HP == 1: w = s
                for i in range(HP):
                    v = w[(-i) % HP]
                    out[i].append(zero_u if v is None else v)
            return [jnp.concatenate(o, axis=0) for o in out]
        def pv(h, ii, p):
            w0 = (20*h)//8*8; off = 20*h - w0
            nk = 384 - 128 * kt_lo
            vt = vT_s[pl.ds(w0, 24), pl.ds(q0 - 256 + 128*kt_lo, nk)]
            grow = 23 if off == 0 else 0
            blk = grow // 8
            parts = [vt[8*t:8*t+8] for t in range(3)]
            parts[blk] = jnp.where(lax.broadcasted_iota(jnp.int32, (8, nk), 0) == grow % 8, 1.0, parts[blk])
            o = dot(jnp.concatenate(parts, axis=0), bc(p))
            o = o * (1.0 / o[grow:grow+1])
            if ii > 0: o = pltpu.roll(o, 128 - NQ*ii, 1)
            return o
        def flush(j, outs):
            o0, o1, o2, o3 = outs
            oT = [o0[0:16], jnp.where(lo4, o0[16:24], o1[0:8]), o1[8:24], o2[0:16], jnp.where(lo4, o2[16:24], o3[0:8]), o3[8:24]]
            oT_s[b % 2, pl.ds(80*j, 80), :] = jnp.concatenate(oT, axis=0)
        sets = [(j, list(range(i0, i0+HP))) for j in range(8) for i0 in range(0, 4, HP)]
        NT_ = len(sets) * HP
        st = {}; ps = {}; R = {}; mg = {}; outs = {}
        nsteps = NT_ + LA + LB + HP
        assert len(extras) == nsteps
        for t in range(nsteps):
            if t < NT_:
                si, a = divmod(t, HP)
                if a == 0: R[si] = make_R(*sets[si])
                st[t] = qk_tile(sets[si][0], a, R[si])
            for f in extras[t]: f()
            u = t - LA
            if 0 <= u < NT_: ps[u] = sm_tile(*st.pop(u))
            v = u - LB - (HP - 1)
            if 0 <= v < NT_:
                si, ii = divmod(v, HP)
                j, heads = sets[si]
                if ii == 0: mg[si] = merge([ps.pop(HP*si + a) for a in range(HP)])
                h = 4*j + heads[ii]
                outs[h] = pv(h, ii, mg[si][ii])
                if h % 4 == 3: flush(j, [outs.pop(4*j + k) for k in range(4)])
    NSTEP = 32 + LA + LB + HP

    def st1(b):
        def f():
            r0 = b * 128
            xt = [ax_v[pl.ds(r0, 128), 128*t:128*t+128].astype(F32) for t in range(5)]
            b_, c_, d_, e_ = xt[1] + xt[4], xt[2] + xt[3], xt[1] - xt[4], xt[2] - xt[3]
            T = [xt[0] + b_ + c_, xt[0] + c1*b_ + c2*c_, -s1*d_ - s2*e_, xt[0] + c2*b_ + c1*c_, s1*e_ - s2*d_]
            for t in range(5):
                for a in range(8):
                    ts[t, pl.ds(8*b + a, 16, stride=P), :] = T[t][16*a:16*a+16]
        return f
    def wprep(k2):
        def f():
            for a, src in enumerate((wr_v, wi_v)):
                wf[a, k2, 0:320, :] = src[0:320, pl.ds(128*k2, 128)].astype(F32)
                wf[a, k2, 320:321, :] = src[320:321, pl.ds(128*k2, 128)].astype(F32)
        return f
    def st2(n2):
        def f():
            base = n2 * P
            T = [ts[t, pl.ds(base, 128), :].astype(BF) for t in range(5)]
            Z0 = ntdot(dm_v[0, 0:128, 0:128], T[0])
            ZA = ntdot(dm_v[1], jnp.concatenate(T[1:3], axis=1))
            ZB = ntdot(dm_v[2], jnp.concatenate(T[3:5], axis=1))
            ZT = jnp.concatenate([Z0, ZA, ZB], axis=0).astype(BF)
            PT = dot(ZT, ft_v[n2])
            g_s[0, n2] = PT[0:128, 0:128]; g_s[1, n2] = PT[0:128, 128:256]
            g_s[2, n2] = PT[128:256, 0:128] - PT[256:384, 128:256]; g_s[3, n2] = PT[128:256, 128:256] + PT[256:384, 0:128]
            g_s[4, n2] = PT[384:512, 0:128] - PT[512:640, 128:256]; g_s[5, n2] = PT[384:512, 128:256] + PT[512:640, 0:128]
        return f
    def ldc(g, pos, r0): return (g_s[2*g, pos, pl.ds(r0, 8), :], g_s[2*g+1, pos, pl.ds(r0, 8), :])
    def stc(g, pos, r0, v):
        g_s[2*g, pos, pl.ds(r0, 8), :] = v[0]
        g_s[2*g+1, pos, pl.ds(r0, 8), :] = v[1]
    def tw(v, n, sign): return cmul_const(v[0], v[1], np.exp(sign * 2j * np.pi * n / 16))
    def p1(g, r0):
        def f():
            for n2 in range(4):
                y = dft4([ldc(g, 4*n1 + n2, r0) for n1 in range(4)], -1)
                for k1 in range(4): stc(g, 4*k1 + n2, r0, tw(y[k1], n2*k1, -1))
        return f
    def mulw(x, k2, wrow, special=None):
        wr = wf[0, k2, pl.ds(wrow, 8, stride=5), :]
        wi = wf[1, k2, pl.ds(wrow, 8, stride=5), :]
        if special is not None:
            wr = jnp.where(special, wf[0, k2, 320:321, :], wr); wi = jnp.where(special, wf[1, k2, 320:321, :], wi)
        return (x[0]*wr - x[1]*wi, x[0]*wi + x[1]*wr)
    def inv1(g, r0, k1, Y):
        u = dft4(Y, +1)
        for j1 in range(4): stc(g, 4*k1 + j1, r0, tw(u[j1], k1*j1, +1))
    def p2ab(g, rr, half):
        def f():
            c = ((1, 4), (2, 3))[g-1][half]
            r0 = rr*8 + 64*half
            for k1 in range(4):
                X = dft4([ldc(g, 4*k1 + n2, r0) for n2 in range(4)], -1)
                inv1(g, r0, k1, [mulw(X[k2], k1 + 4*k2, 40*rr + c) for k2 in range(4)])
        return f
    def p2g0(rr):
        def f():
            r0, r1 = rr*8, rr*8 + 64
            for k1 in range(4):
                Xa = dft4([ldc(0, 4*k1 + n2, r0) for n2 in range(4)], -1)
                Xb = dft4([ldc(0, 4*k1 + n2, r1) for n2 in range(4)], -1)
                Ya, Yb = [], []
                for k2 in range(4):
                    ar, ai = Xa[k2]; br, bi = Xb[k2]
                    if rr == 0:
                        keep = row8 == 0
                        A2 = (jnp.where(keep, ar, ar - bi), jnp.where(keep, ai, ai + br))
                        B2 = (jnp.where(keep, br, br + ai), jnp.where(keep, bi, bi - ar))
                    else:
                        A2 = (ar - bi, ai + br); B2 = (br + ai, bi - ar)
                    Ya.append(mulw(A2, k1 + 4*k2, 40*rr))
                    Yb.append(mulw(B2, k1 + 4*k2, 40*rr, special=(row8 == 0) if rr == 0 else None))
                inv1(0, r0, k1, Ya); inv1(0, r1, k1, Yb)
        return f
    def p3(g, rp):
        def f():
            for j1 in range(4):
                ua = dft4([ldc(g, 4*k1 + j1, 16*rp) for k1 in range(4)], +1)
                ub = dft4([ldc(g, 4*k1 + j1, 16*rp + 8) for k1 in range(4)], +1)
                for j2 in range(4):
                    m2 = j1 + 4*j2
                    u_s[2*g, m2, pl.ds(8*rp, 8), :] = pk2(ua[j2][0], ub[j2][0])
                    u_s[2*g+1, m2, pl.ds(8*rp, 8), :] = pk2(ua[j2][1], ub[j2][1])
        return f
    def st3_items(rr):
        it = []
        for g in range(3):
            it += [p1(g, 8*rr), p1(g, 8*rr + 64)]
        it += [p2ab(1, rr, 0), p2ab(1, rr, 1), p2g0(rr), p2ab(2, rr, 0), p2ab(2, rr, 1)]
        return it
    def st3_fin(rr):
        return [p3(g, rp) for g in range(3) for rp in (rr//2, 4 + rr//2)]
    def st4(m2):
        def f():
            hm = hs_v[m2]
            rhs = bc(jnp.concatenate([u_s[k, m2] for k in range(2, 6)], axis=0))
            Q = ntdot(hm, rhs)
            Qr, Qi = Q[:128], Q[128:]
            z0 = ntdot(hm[:128], bc(u_s[0, m2])) - ntdot(hm[128:], bc(u_s[1, m2]))
            zA = jnp.concatenate([Qr[:, 0:128] - Qi[:, 128:256], Qi[:, 0:128] + Qr[:, 128:256]], axis=1).astype(BF)
            zB = jnp.concatenate([Qr[:, 256:384] - Qi[:, 384:512], Qi[:, 256:384] + Qr[:, 384:512]], axis=1).astype(BF)
            V0 = dot(z0.astype(BF), dm_v[3, 0:128, 0:128])
            U1 = dot(zA, dm_v[4]); U2 = dot(zB, dm_v[5])
            U1r, U1i, U2r, U2i = U1[:, :128], U1[:, 128:], U2[:, :128], U2[:, 128:]
            p = V0 + c1*U1r + c2*U2r; q = s1*U1i + s2*U2i
            pp = V0 + c2*U1r + c1*U2r; qq = s2*U1i - s1*U2i
            y = [V0 + U1r + U2r, p - q, pp - qq, pp + qq, p + q]
            for t in range(5):
                ts[t, pl.ds(m2 * P, 128), :] = y[t]
        return f
    def st5(b):
        def f():
            for t in range(5):
                z = jnp.concatenate([ts[t, pl.ds(8*b + a, 16, stride=P), :] for a in range(8)], axis=0)
                outa_v[pl.ds(b*128, 128), 128*t:128*t+128] = z.astype(BF)
            out_a(b).start()
        return f

    p0, p1_ = proj_items(0), proj_items(1)
    with scope("pro_wait0"):
        cp_x(0).wait()
        for n in WORDER[0:5]: cp_w(n).wait()
    for n in WORDER[10:15]: cp_w(n).start()
    cp_x(1).start()
    with scope("pro_c0"):
        for n in WORDER[0:5]:
            for f in p0[n] + p1_[n]: f()
    with scope("pro_w1"):
        for n in WORDER[5:10]: cp_w(n).wait()
    cp_a(0).start()
    with scope("pro_c1"):
        for n in WORDER[5:10]:
            for f in p0[n] + p1_[n]: f()
    with scope("pro_w2"):
        for n in WORDER[10:15]: cp_w(n).wait()
    cp_a(1).start(); cp_wo.start()
    with scope("pro_c2"):
        for n in WORDER[10:15]:
            for f in p0[n] + p1_[n]: f()
    def spread(items, lo, hi, ex):
        n = hi - lo
        for k, f in enumerate(items): ex[lo + k * n // max(len(items), 1)].append(f)
    for b in range(NB):
        ex = [[] for _ in range(NSTEP)]
        aitems = []
        if b == 0:
            with scope("w_it0"):
                cp_x(1).wait(); cp_a(0).wait()
            cp_dm.start(); cp_ft.start()
            aitems = [st1(k) for k in range(0, 8)]
        elif b == 1:
            with scope("w_it1"):
                cp_a(1).wait(); cp_wo.wait()
            cp_wr.start(); cp_wi.start(); cp_x(2).start()
            aitems = [st1(k) for k in range(8, 16)]
        elif 2 <= b <= 5:
            if b == 2:
                with scope("w_it2"):
                    for c in (cp_dm, cp_ft, cp_wr, cp_wi, cp_x(2)): c.wait()
                cp_hs.start(); cp_x(3).start(); cp_x(4).start()
            if b == 4:
                with scope("w_it4"):
                    for c in (cp_x(3), cp_x(4), cp_hs): c.wait()
            k = b - 2
            aitems = [st2(4*k), wprep(4*k), wprep(4*k+1), st2(4*k+1), wprep(4*k+2), st2(4*k+2), wprep(4*k+3), st2(4*k+3)]
        elif 6 <= b <= 9:
            k = b - 6
            aitems = st3_items(2*k) + st3_items(2*k + 1) + st3_fin(2*k + 1)
        elif 10 <= b <= 13:
            aitems = [st4(4*(b-10) + k) for k in range(4)]
        elif b == 14: aitems = [st5(k) for k in range(0, 8)]
        elif b == 15: aitems = [st5(k) for k in range(8, 16)]
        spread(aitems, 0, NSTEP, ex)
        if b > 0: spread(outproj_items(b - 1), 0, E("ES", 16), ex)
        if b + 2 < NB:
            pi = proj_items(b + 2)
            spread([f for n in WORDER for f in pi[n]], E("PS", 8), NSTEP, ex)
        with scope(f'it{b:02d}'):
            attn(b, ex)
    with scope('epi'):
        for f in outproj_items(NB - 1): f()
    with scope('epi_wait'):
        for b in range(NB): out_b(b).wait()
        for b in range(NB): out_a(b).wait()

_DM, _FT, _HS = a_consts3()

@jax.jit
def pallas_concat_heads__spectral_gfnet__sliding_block__prompt_kernel(A_x, A_w_r, A_w_i, B_x, B_wqkv, B_wo):
    anyspec = pl.BlockSpec(memory_space=pl.ANY)
    V = pltpu.VMEM
    return pl.pallas_call(
        kernel,
        out_shape=jax.ShapeDtypeStruct((1, S, 2*D), BF),
        in_specs=[anyspec]*9, out_specs=anyspec,
        scratch_shapes=[
            V((S, D), BF), V((DF, S), BF), V((DF, S), BF), V((16, 128, 256), BF), V((16, 256, 128), BF), V((6, 256, 256), BF),
            V((5, 16*P, 128), F32), V((6, 16, 128, 128), F32), V((6, 16, 64, 128), U32), V((2, 16, 328, 128), F32), V((S, D), BF),
            V((S, D), BF), V((D, 3*D), BF), V((D, D), BF),
            V((8, S//2, 128), U32), V((D//2, S), U32), V((D, S), F32), V((2, D, 128), F32), V((S, D), BF),
            V((2, 5, 64, 128), U32), V((64, D), U32),
            pltpu.SemaphoreType.DMA((16,)), pltpu.SemaphoreType.DMA((5,)), pltpu.SemaphoreType.DMA((7,)),
            pltpu.SemaphoreType.DMA(()), pltpu.SemaphoreType.DMA(()),
        ],
        compiler_params=pltpu.CompilerParams(vmem_limit_bytes=120*2**20),
        name="kF",
    )(A_x, A_w_r.T, A_w_i.T, B_x, B_wqkv, B_wo, jnp.asarray(_FT), jnp.asarray(_HS), jnp.asarray(_DM))
```

```python
import contextlib
def scope(n): return contextlib.nullcontext()
import numpy as np
import ml_dtypes
import jax
import jax.numpy as jnp
from jax import lax
from jax.experimental import pallas as pl
from jax.experimental.pallas import tpu as pltpu
BFn = ml_dtypes.bfloat16

S, D, H, DH = 2048, 640, 32, 20
DF = 321
BQ = 128
NB = S // BQ
BF, F32, U32 = jnp.bfloat16, jnp.float32, jnp.uint32
QSCALE = float(DH ** -0.5 * np.log2(np.e))
NEG = -1e30
P = 132
c1, c2, s1, s2 = (float(np.cos(2*np.pi/5)), float(np.cos(4*np.pi/5)), float(np.sin(2*np.pi/5)), float(np.sin(4*np.pi/5)))
E = lambda k, d: d
HP = E("HP", 2); LA = E("LA", 1); LB = E("LB", 3)
NQ = 128 // HP; NP = NQ // 16; NMID = (256 - NQ) // 16; NGRP = 2*NP + NMID
NT = (((1,), (1,)), ((), ()))
def freq_lanes(c):
    l = np.arange(128)
    return np.where(l < 64, 5*l + c, 5*(l-64) + (5-c))
def d_mats():
    d1 = np.arange(128)[:, None].astype(np.float64)
    out = []
    for c in (1, 2):
        f = freq_lanes(c)[None, :].astype(np.float64)
        sg = np.where(np.arange(128)[None, :] < 64, 1.0, -1.0)
        C = np.cos(2*np.pi*f*d1/D); Sn = -np.sin(2*np.pi*f*d1/D)
        M = np.zeros((256, 256))
        M[:128, :128] = C; M[128:, :128] = -sg*Sn; M[:128, 128:] = Sn; M[128:, 128:] = sg*C
        out.append(M)
    l = np.arange(128)[None, :]
    fre = 5.0*l; fim = 5.0*(l-64)
    M0 = np.where(l <= 64, np.cos(2*np.pi*fre*d1/D), -np.sin(2*np.pi*fim*d1/D))
    MA, MB = out
    IA = MA.T*2.0/D; IB = MB.T*2.0/D
    cf = np.where((l == 0) | (l == 64), 1.0, 2.0)
    I0 = (M0*cf).T / D
    return M0, MA, MB, I0, IA, IB
def s_mats():
    k1 = np.arange(128)[:, None]; n1 = np.arange(128)[None, :]
    F = np.zeros((16, 256, 128)); Hh = np.zeros((16, 256, 128))
    for n2 in range(16):
        ph = 2*np.pi*((k1*(16*n1+n2)) % S)/S
        F[n2, :128] = np.cos(ph); F[n2, 128:] = -np.sin(ph)
        Hh[n2, :128] = np.cos(ph).T/S; Hh[n2, 128:] = np.sin(ph).T/S
    return F, Hh
def a_consts2():
    M0, MA, MB, I0, IA, IB = d_mats()
    dm = np.zeros((6, 256, 256), np.float32)
    dm[0, :128, :128] = M0.T; dm[1] = MA.T; dm[2] = MB.T
    dm[3, :128, :128] = I0; dm[4] = IA; dm[5] = IB
    F, Hh = s_mats()
    FT = np.concatenate([F[:, :128].transpose(0, 2, 1), F[:, 128:].transpose(0, 2, 1)], axis=2)
    return dm.astype(BFn), FT.astype(np.float32).astype(BFn), Hh.astype(np.float32).astype(BFn)

def a_consts3():
    dm, FT, HS = a_consts2()
    perm = np.arange(128).reshape(8, 2, 8).transpose(0, 2, 1).reshape(128)
    dm = dm.copy()
    dm[3, :128] = dm[3, :128][perm]
    for k in (4, 5):
        dm[k, :128] = dm[k, :128][perm]
        dm[k, 128:] = dm[k, 128:][perm]
    return dm, FT, HS

def cmul_const(ar, ai, w):
    wr_, wi_ = round(w.real, 12), round(w.imag, 12)
    if wi_ == 0 and wr_ == 1: return ar, ai
    if wi_ == 0 and wr_ == -1: return -ar, -ai
    if wr_ == 0 and wi_ == 1: return -ai, ar
    if wr_ == 0 and wi_ == -1: return ai, -ar
    if abs(abs(wr_) - abs(wi_)) < 1e-12:
        k = abs(wr_); sr, si = np.sign(wr_), np.sign(wi_)
        if sr > 0 and si > 0: return (ar - ai)*k, (ar + ai)*k
        if sr > 0 and si < 0: return (ar + ai)*k, (ai - ar)*k
        if sr < 0 and si > 0: return (ar + ai)*(-k), (ar - ai)*k
        return (ai - ar)*k, (ar + ai)*(-k)
    return ar*wr_ - ai*wi_, ar*wi_ + ai*wr_

def dft4(x, sign):
    (ar, ai), (br, bi), (cr, ci), (dr, di) = x
    t0r, t0i = ar + cr, ai + ci
    t1r, t1i = ar - cr, ai - ci
    t2r, t2i = br + dr, bi + di
    t3r, t3i = br - dr, bi - di
    if sign < 0:
        x1 = (t1r + t3i, t1i - t3r); x3 = (t1r - t3i, t1i + t3r)
    else:
        x1 = (t1r - t3i, t1i + t3r); x3 = (t1r + t3i, t1i - t3r)
    return [(t0r + t2r, t0i + t2i), x1, (t0r - t2r, t0i - t2i), x3]

def dft16(x, sign):
    cols = []
    for n2 in range(4):
        y = dft4([x[4*n1 + n2] for n1 in range(4)], sign)
        y = [cmul_const(y[k1][0], y[k1][1], np.exp(sign*2j*np.pi*n2*k1/16)) for k1 in range(4)]
        cols.append(y)
    out = [None]*16
    for k1 in range(4):
        z = dft4([cols[n2][k1] for n2 in range(4)], sign)
        for k2 in range(4): out[k1 + 4*k2] = z[k2]
    return out


def ntdot(a, b): return lax.dot_general(a, b, NT, preferred_element_type=F32)
def dot(a, b): return jnp.dot(a, b, preferred_element_type=F32)
def bc(x): return pltpu.bitcast(x, BF)
def pk2(a, b): return pltpu.pack_elementwise([a, b], packed_dtype=BF)
def tree(xs, f):
    xs = list(xs)
    while len(xs) > 1:
        xs = [f(xs[k], xs[k+1]) if k + 1 < len(xs) else xs[k] for k in range(0, len(xs), 2)]
    return xs[0]
def split_pieces(groups, firsts, lasts, flip):
    units = [[f, l] for f, l in zip(firsts, lasts) if f in groups and l in groups]
    paired = {g for u in units for g in u}
    singles = [g for g in groups if g not in paired]
    n = len(groups)
    sizes = [n // 4] * 4
    order = [2, 3, 0, 1] if flip else [0, 1, 2, 3]
    for k in range(n - sum(sizes)): sizes[order[k]] += 1
    pcs = [[] for _ in range(4)]
    k = 0
    for u in units:
        tries = 0
        while len(pcs[k]) + 2 > sizes[k] and tries < 4: k = (k + 1) % 4; tries += 1
        if tries == 4: singles += u; continue
        pcs[k] += u; k = (k + 1) % 4
    for k in range(4):
        while len(pcs[k]) < sizes[k]: pcs[k].append(singles.pop(0))
    assert not singles
    return [p for p in pcs if p]

def kernel(ax_hbm, wr_hbm, wi_hbm, bx_hbm, wqkv_hbm, wo_hbm, ft_hbm, hs_hbm, dm_hbm, out_hbm,
           ax_v, wr_v, wi_v, ft_v, hs_v, dm_v, ts, g_s, u_s, wf, outa_v,
           bx_v, wqkv_v, wo_v, kg_s, qT_s, vT_s, oT_s, outb_v, kt_s, ol_s,
           sem_w, sem_x, sem_a, sem_outa, sem_outb, sem_bar):
    WORDER = [5, 6, 7, 8, 9, 0, 1, 2, 3, 4, 10, 11, 12, 13, 14]
    def cp_w(n): return pltpu.make_async_copy(wqkv_hbm.at[:, pl.ds(128*n, 128)], wqkv_v.at[:, pl.ds(128*n, 128)], sem_w.at[n])
    def cp_wg(g): return pltpu.make_async_copy(wqkv_hbm.at[:, pl.ds(640*g, 640)], wqkv_v.at[:, pl.ds(640*g, 640)], sem_w.at[g])
    XCH = [(0, 128), (128, 256), (256, 512), (512, 1024), (1024, 1536), (1536, 2048)]
    def cp_x(c):
        lo, hi = XCH[c]
        return pltpu.make_async_copy(bx_hbm.at[0, pl.ds(lo, hi - lo), :], bx_v.at[pl.ds(lo, hi - lo), :], sem_x.at[c])
    ACH = [(0, 1024), (1024, 2048)]
    def cp_a(c):
        lo, hi = ACH[c]
        return pltpu.make_async_copy(ax_hbm.at[0, pl.ds(lo, hi - lo), :], ax_v.at[pl.ds(lo, hi - lo), :], sem_a.at[c])
    cp_wr = pltpu.make_async_copy(wr_hbm, wr_v, sem_a.at[2])
    cp_wi = pltpu.make_async_copy(wi_hbm, wi_v, sem_a.at[3])
    cp_ft = pltpu.make_async_copy(ft_hbm, ft_v, sem_a.at[4])
    cp_hs = pltpu.make_async_copy(hs_hbm, hs_v, sem_a.at[5])
    cp_dm = pltpu.make_async_copy(dm_hbm, dm_v, sem_a.at[6])
    cp_wo = pltpu.make_async_copy(wo_hbm, wo_v, sem_w.at[15])
    cp_x(0).start(); cp_x(1).start()
    cp_wg(1).start()
    cp_wg(0).start()

    row8 = lax.broadcasted_iota(jnp.int32, (8, 128), 0)
    col8 = lax.broadcasted_iota(jnp.int32, (8, 128), 1)
    col64 = lax.broadcasted_iota(jnp.int32, (64, 128), 1)
    DQ = row8 - (col8 & (NQ - 1))
    lo4 = row8 < 4
    part = col8 >> int(np.log2(NQ)) if HP > 1 else col8 * 0
    bits = [((part >> k) & 1) == 1 for k in range(int(np.log2(HP)))]
    zero_u = jnp.zeros((8, 128), U32)

    anc = {'z': None}
    PACE = "13w"
    def zvec():
        k = min(anc['k'], 15); anc['k'] += E("PSTEP", 3)
        y = anc['src'][8*k:8*k+8]
        return y - y
    def pace(x, st):
        return x if (anc['z'] is None or st not in PACE) else x + zvec()
    def pace_u(x, n, st):
        if anc['z'] is None or st not in PACE: return x
        z = pltpu.bitcast(zvec(), U32)
        return jnp.concatenate([x[0:8] | z, x[8:n]], axis=0)
    def proj_items(b):
        r0 = b * BQ; u0 = b * 64
        def mm(n):
            y = dot(bx_v[pl.ds(r0, BQ), :], wqkv_v[:, 128*n:128*n+128])
            if PACE: anc['src'] = y; anc['k'] = 0; anc['z'] = True
            return y
        def qtile(t):
            def f():
                q = (mm(t) * QSCALE).astype(BF)
                qT_s[64*t:64*t+64, pl.ds(r0, BQ)] = pltpu.bitcast(q.T, U32)
            return f
        def vtile(t):
            def f():
                v = mm(10 + t)
                w = pk2(jnp.concatenate([v[16*g:16*g+8] for g in range(8)], axis=0),
                        jnp.concatenate([v[16*g+8:16*g+16] for g in range(8)], axis=0))
                vT_s[128*t:128*t+128, pl.ds(r0, BQ)] = bc(w).T.astype(F32)
            return f
        def ktile(t):
            def f(): kt_s[b % 2, t] = pltpu.bitcast(mm(5 + t).astype(BF), U32)
            return f
        def kgrp(j):
            def f():
                t0, off = divmod(80 * j, 128)
                a = kt_s[b % 2, t0]
                if off > 0: a = pltpu.roll(a, 128 - off, 1)
                if off + 80 > 128:
                    a = jnp.where(col64 < 128 - off, a, pltpu.roll(kt_s[b % 2, t0 + 1], 128 - off, 1))
                kg_s[j, pl.ds(u0, 64), :] = jnp.where(col64 < 80, a, U32(0))
            return f
        by_tile = {5: [ktile(0), kgrp(0)], 6: [ktile(1), kgrp(1), kgrp(2)], 7: [ktile(2), kgrp(3)], 8: [ktile(3), kgrp(4), kgrp(5)], 9: [ktile(4), kgrp(6), kgrp(7)]}
        for t in range(5):
            by_tile[t] = [qtile(t)]; by_tile[10 + t] = [vtile(t)]
        return by_tile

    def outproj_items(b):
        r0 = b * BQ
        def tr(t):
            def f(): ol_s[b % 2, :, 128*t:128*t+128] = oT_s[b, 128*t:128*t+128, :].astype(BF).T
            return f
        def mm(n):
            def f(): outb_v[pl.ds(r0, BQ), 128*n:128*n+128] = dot(ol_s[b % 2], wo_v[:, 128*n:128*n+128]).astype(BF)
            return f
        def dma():
            out_b(b).start()
        return [tr(t) for t in range(5)] + [mm(n) for n in range(5)] + [dma]
    def out_b(b):
        return pltpu.make_async_copy(outb_v.at[pl.ds(b*BQ, BQ), :], out_hbm.at[0, pl.ds(b*BQ, BQ), pl.ds(D, D)], sem_outb)
    def out_a(b):
        return pltpu.make_async_copy(outa_v.at[pl.ds(b*BQ, BQ), :], out_hbm.at[0, pl.ds(b*BQ, BQ), pl.ds(0, D)], sem_outa)

    def attn_ctx(b):
        q0 = b * 128
        def make_R(j, heads):
            R = {}
            for ii, i in enumerate(heads):
                lo, hi = 10*i, 10*i + 10
                for t in range(lo//8, (hi-1)//8 + 1):
                    q = qT_s[pl.ds(40*j + 8*t, 8), pl.ds(q0, 128)]
                    if ii > 0: q = pltpu.roll(q, NQ*ii, 1)
                    rlo, rhi = max(lo - 8*t, 0), min(hi - 8*t, 8)
                    R.setdefault(t, []).append((ii, q, rlo, rhi))
            return R
        def make_qm(R, a):
            out = []
            for t in range(5):
                if t not in R: out.append(zero_u); continue
                v = zero_u
                for (ii, q, rlo, rhi) in R[t]:
                    full = (rlo == 0 and rhi == 8)
                    msk = None if full else ((row8 >= rlo) & (row8 < rhi))
                    if HP > 1:
                        pm = part == (ii + a) % HP
                        msk = pm if msk is None else (msk & pm)
                    v = q if msk is None else jnp.where(msk, q, v)
                out.append(v)
            return bc(jnp.concatenate(out, axis=0))
        def key0(a): return q0 - 256 + NQ * a
        def valid(a):
            return [g for g in range(NGRP) if key0(a) + 16*g >= 0]
        def qk_tile(j, a, R):
            qm = make_qm(R, a)
            base = (key0(a)) // 2
            def rows(ids): return bc(jnp.concatenate([kg_s[j, pl.ds(base + 8*g, 8), :] for g in ids], axis=0))[:, 0:80]
            vals = {}
            for ids in split_pieces(valid(a), list(range(NP)), list(range(NP + NMID, NGRP)), a % 2):
                s = dot(rows(ids), qm)
                for n, g in enumerate(ids):
                    vals[g] = (s[16*n:16*n+8], s[16*n+8:16*n+16])
            cs = []
            for r in range(2*NP):
                g, hh = divmod(r, 2)
                fst = vals[g][hh] if g in vals else NEG
                cs.append(jnp.where(DQ > -8*r, fst, vals[NP + NMID + g][hh]))
            mid = {g: vals[g] for g in range(NP, NP + NMID) if g in vals}
            return cs, mid, [g in vals for g in range(NP)]
        def sm_tile(cs, mid, has_first):
            allv = cs + [x for g in mid for x in mid[g]]
            m8 = tree(allv, jnp.maximum)
            if 'a' in PACE: anc['src'] = jnp.concatenate([m8] * 16, axis=0); anc['k'] = 0; anc['z'] = True
            m = jnp.max(m8, axis=0, keepdims=True)
            pc = [jnp.exp2(c - m) for c in cs]
            Pg = {}
            for g in range(NP):
                if has_first[g]:
                    p0 = [jnp.where(DQ > -8*(2*g + hh), pc[2*g + hh], 0.0) for hh in range(2)]
                    Pg[g] = pk2(p0[0], p0[1])
                    Pg[NP + NMID + g] = pk2(pc[2*g] - p0[0], pc[2*g + 1] - p0[1])
                else:
                    Pg[NP + NMID + g] = pk2(pc[2*g], pc[2*g + 1])
            for g in mid:
                Pg[g] = pk2(jnp.exp2(mid[g][0] - m), jnp.exp2(mid[g][1] - m))
            return Pg
        kt_lo = max(0, (256 - q0) // 128)
        def merge(Ps):
            out = [[] for _ in range(HP)]
            for gam in range(8 * kt_lo, 24):
                s = [Ps[a].get(gam - NP*a) if 0 <= gam - NP*a < NGRP else None for a in range(HP)]
                def sel(mask, x, y):
                    if x is None and y is None: return None
                    return jnp.where(mask, zero_u if x is None else x, zero_u if y is None else y)
                w = s
                for k, bit in enumerate(bits):
                    w = [sel(bit, w[(n + (1 << k)) % HP], w[n]) for n in range(HP)]
                if HP == 1: w = s
                for i in range(HP):
                    v = w[(-i) % HP]
                    out[i].append(zero_u if v is None else v)
            return [jnp.concatenate(o, axis=0) for o in out]
        def pv(h, ii, p):
            w0 = (20*h)//8*8; off = 20*h - w0
            nk = 384 - 128 * kt_lo
            vt = vT_s[pl.ds(w0, 24), pl.ds(q0 - 256 + 128*kt_lo, nk)]
            grow = 23 if off == 0 else 0
            blk = grow // 8
            parts = [vt[8*t:8*t+8] for t in range(3)]
            parts[blk] = jnp.where(lax.broadcasted_iota(jnp.int32, (8, nk), 0) == grow % 8, 1.0, parts[blk])
            o = dot(jnp.concatenate(parts, axis=0), bc(p))
            o = o * (1.0 / o[grow:grow+1])
            if ii > 0: o = pltpu.roll(o, 128 - NQ*ii, 1)
            return o
        def flush(j, outs):
            o0, o1, o2, o3 = outs
            oT = [o0[0:16], jnp.where(lo4, o0[16:24], o1[0:8]), o1[8:24], o2[0:16], jnp.where(lo4, o2[16:24], o3[0:8]), o3[8:24]]
            oT_s[b, pl.ds(80*j, 80), :] = jnp.concatenate(oT, axis=0)
        return make_R, qk_tile, sm_tile, merge, pv, flush
    sets = [(j, list(range(i0, i0+HP))) for j in range(8) for i0 in range(0, 4, HP)]
    NT_ = len(sets) * HP
    def attn_flow(blocks, extras, marks=None):
        ctx = {b: attn_ctx(b) for b in blocks}
        tiles = [(b, t) for b in blocks for t in range(NT_)]
        n = len(tiles)
        st = {}; ps = {}; R = {}; mg = {}; outs = {}
        for g in range(n + LA + LB + HP):
            if g < n:
                b, t = tiles[g]
                if t == 0 and marks: marks(b)
                si, a = divmod(t, HP)
                if a == 0: R[(b, si)] = ctx[b][0](*sets[si])
                st[g] = ctx[b][1](sets[si][0], a, R[(b, si)])
                if a == HP - 1: R.pop((b, si))
                for f in extras[b][t]: f()
            u = g - LA
            if 0 <= u < n: ps[u] = ctx[tiles[u][0]][2](*st.pop(u))
            v = g - LB - (HP - 1)
            if 0 <= v < n:
                b, t = tiles[v]
                si, ii = divmod(t, HP)
                j, heads = sets[si]
                if ii == 0: mg[v] = ctx[b][3]([ps.pop(v + a) for a in range(HP)])
                h = 4*j + heads[ii]
                outs[(b, h)] = ctx[b][4](h, ii, mg[v - ii][ii])
                if ii == HP - 1: mg.pop(v - ii)
                if h % 4 == 3: ctx[b][5](j, [outs.pop((b, 4*j + k)) for k in range(4)])

    def st1(b):
        def piece(a):
            def f():
                r0 = b * 128 + 16 * a
                xt = [ax_v[pl.ds(r0, 16), 128*t:128*t+128].astype(F32) for t in range(5)]
                if '1' in PACE and anc['z'] is not None:
                    z2 = jnp.concatenate([zvec()] * 2, axis=0)
                    xt[1] = xt[1] + z2; xt[2] = xt[2] + z2
                b_, c_, d_, e_ = xt[1] + xt[4], xt[2] + xt[3], xt[1] - xt[4], xt[2] - xt[3]
                T = [xt[0] + b_ + c_, xt[0] + c1*b_ + c2*c_, -s1*d_ - s2*e_, xt[0] + c2*b_ + c1*c_, s1*e_ - s2*d_]
                for t in range(5):
                    ts[t, pl.ds(8*b + a, 16, stride=P), :] = T[t]
            return f
        return [piece(a) for a in range(8)]
    def wprep(k2):
        def f():
            for a, src in enumerate((wr_v, wi_v)):
                for r in range(0, 320, 32):
                    w = src[r:r+32, pl.ds(128*k2, 128)].astype(F32)
                    if 'w' in PACE and anc['z'] is not None: w = w + jnp.concatenate([zvec()] * 4, axis=0)
                    wf[a, k2, r:r+32, :] = w
                wf[a, k2, 320:321, :] = src[320:321, pl.ds(128*k2, 128)].astype(F32)
        return f
    def st2(n2):
        base = n2 * P
        def ldT(t): return ts[t, pl.ds(base, 128), :].astype(BF)
        V2 = E("V2", 0)
        def whole():
            T = [ldT(t) for t in range(5)]
            Z0 = ntdot(dm_v[0, 0:128, 0:128], T[0])
            ZA = ntdot(dm_v[1], jnp.concatenate(T[1:3], axis=1))
            ZB = ntdot(dm_v[2], jnp.concatenate(T[3:5], axis=1))
            ZT = jnp.concatenate([Z0, ZA, ZB], axis=0).astype(BF)
            PT = dot(ZT, ft_v[n2])
            g_s[0, n2] = PT[0:128, 0:128]; g_s[1, n2] = PT[0:128, 128:256]
            g_s[2, n2] = PT[128:256, 0:128] - PT[256:384, 128:256]; g_s[3, n2] = PT[128:256, 128:256] + PT[256:384, 0:128]
            g_s[4, n2] = PT[384:512, 0:128] - PT[512:640, 128:256]; g_s[5, n2] = PT[384:512, 128:256] + PT[512:640, 0:128]
        def g0():
            z = ntdot(dm_v[0, 0:128, 0:128], ldT(0)).astype(BF)
            PT = dot(z, ft_v[n2])
            g_s[0, n2] = PT[:, 0:128]; g_s[1, n2] = PT[:, 128:256]
        def gab(g):
            def f():
                Z = ntdot(dm_v[g], jnp.concatenate([ldT(2*g - 1), ldT(2*g)], axis=1)).astype(BF)
                PT = dot(Z, ft_v[n2])
                g_s[2*g, n2] = PT[0:128, 0:128] - PT[128:256, 128:256]
                g_s[2*g + 1, n2] = PT[0:128, 128:256] + PT[128:256, 0:128]
            return f
        return [whole] if V2 == 0 else [g0, gab(1), gab(2)]
    def ldc(g, pos, r0): return (g_s[2*g, pos, pl.ds(r0, 8), :], g_s[2*g+1, pos, pl.ds(r0, 8), :])
    def stc(g, pos, r0, v):
        g_s[2*g, pos, pl.ds(r0, 8), :] = v[0]
        g_s[2*g+1, pos, pl.ds(r0, 8), :] = v[1]
    def tw(v, n, sign): return cmul_const(v[0], v[1], np.exp(sign * 2j * np.pi * n / 16))
    def p1(g, r0):
        def one(n2):
            def f():
                xs = [ldc(g, 4*n1 + n2, r0) for n1 in range(4)]
                xs[0] = (pace(xs[0][0], '3'), xs[0][1])
                y = dft4(xs, -1)
                for k1 in range(4): stc(g, 4*k1 + n2, r0, tw(y[k1], n2*k1, -1))
            return f
        return [one(n2) for n2 in range(4)]
    def mulw(x, k2, wrow, special=None):
        wr = wf[0, k2, pl.ds(wrow, 8, stride=5), :]
        wi = wf[1, k2, pl.ds(wrow, 8, stride=5), :]
        if special is not None:
            wr = jnp.where(special, wf[0, k2, 320:321, :], wr); wi = jnp.where(special, wf[1, k2, 320:321, :], wi)
        return (x[0]*wr - x[1]*wi, x[0]*wi + x[1]*wr)
    def inv1(g, r0, k1, Y):
        u = dft4(Y, +1)
        for j1 in range(4): stc(g, 4*k1 + j1, r0, tw(u[j1], k1*j1, +1))
    def p2ab(g, rr, half):
        c = ((1, 4), (2, 3))[g-1][half]
        r0 = rr*8 + 64*half
        def one(k1):
            def f():
                xs = [ldc(g, 4*k1 + n2, r0) for n2 in range(4)]
                xs[0] = (pace(xs[0][0], '3'), xs[0][1])
                X = dft4(xs, -1)
                inv1(g, r0, k1, [mulw(X[k2], k1 + 4*k2, 40*rr + c) for k2 in range(4)])
            return f
        return [one(k1) for k1 in range(4)]
    def p2g0(rr):
        r0, r1 = rr*8, rr*8 + 64
        def one(k1):
            def f():
                xa = [ldc(0, 4*k1 + n2, r0) for n2 in range(4)]; xb = [ldc(0, 4*k1 + n2, r1) for n2 in range(4)]
                xa[0] = (pace(xa[0][0], '3'), xa[0][1]); xb[0] = (pace(xb[0][0], '3'), xb[0][1])
                Xa = dft4(xa, -1); Xb = dft4(xb, -1)
                Ya, Yb = [], []
                for k2 in range(4):
                    ar, ai = Xa[k2]; br, bi = Xb[k2]
                    if rr == 0:
                        keep = row8 == 0
                        A2 = (jnp.where(keep, ar, ar - bi), jnp.where(keep, ai, ai + br))
                        B2 = (jnp.where(keep, br, br + ai), jnp.where(keep, bi, bi - ar))
                    else:
                        A2 = (ar - bi, ai + br); B2 = (br + ai, bi - ar)
                    Ya.append(mulw(A2, k1 + 4*k2, 40*rr))
                    Yb.append(mulw(B2, k1 + 4*k2, 40*rr, special=(row8 == 0) if rr == 0 else None))
                inv1(0, r0, k1, Ya); inv1(0, r1, k1, Yb)
            return f
        return [one(k1) for k1 in range(4)]
    def p3(g, rp):
        def one(j1):
            def f():
                xa = [ldc(g, 4*k1 + j1, 16*rp) for k1 in range(4)]; xb = [ldc(g, 4*k1 + j1, 16*rp + 8) for k1 in range(4)]
                xa[0] = (pace(xa[0][0], '3'), xa[0][1]); xb[0] = (pace(xb[0][0], '3'), xb[0][1])
                ua = dft4(xa, +1); ub = dft4(xb, +1)
                for j2 in range(4):
                    m2 = j1 + 4*j2
                    u_s[2*g, m2, pl.ds(8*rp, 8), :] = pk2(ua[j2][0], ub[j2][0])
                    u_s[2*g+1, m2, pl.ds(8*rp, 8), :] = pk2(ua[j2][1], ub[j2][1])
            return f
        return [one(j1) for j1 in range(4)]
    def st3_items(rr):
        it = []
        for g in range(3):
            it += p1(g, 8*rr) + p1(g, 8*rr + 64)
        it += p2ab(1, rr, 0) + p2ab(1, rr, 1) + p2g0(rr) + p2ab(2, rr, 0) + p2ab(2, rr, 1)
        return it
    def st3_fin(rr):
        return [f for g in range(3) for rp in (rr//2, 4 + rr//2) for f in p3(g, rp)]
    def st4(m2):
        zz = {}
        def hr(): return hs_v[m2, 0:128, :]
        def hi(): return hs_v[m2, 128:256, :]
        def z0():
            zz[0] = (ntdot(hr(), bc(u_s[0, m2])) - ntdot(hi(), bc(u_s[1, m2]))).astype(BF)
        def zab(g):
            def f():
                ur, ui = bc(u_s[2*g, m2]), bc(u_s[2*g + 1, m2])
                zr = ntdot(hr(), ur) - ntdot(hi(), ui)
                zi = ntdot(hi(), ur) + ntdot(hr(), ui)
                zz[g] = jnp.concatenate([zr, zi], axis=1).astype(BF)
            return f
        def dinv(h):
            def f():
                rows = slice(64*h, 64*h + 64)
                V0 = dot(zz[0][rows], dm_v[3, 0:128, 0:128])
                U1 = dot(zz[1][rows], dm_v[4]); U2 = dot(zz[2][rows], dm_v[5])
                U1r, U1i, U2r, U2i = U1[:, :128], U1[:, 128:], U2[:, :128], U2[:, 128:]
                p = V0 + c1*U1r + c2*U2r; q = s1*U1i + s2*U2i
                pp = V0 + c2*U1r + c1*U2r; qq = s2*U1i - s1*U2i
                y = [V0 + U1r + U2r, p - q, pp - qq, pp + qq, p + q]
                for t in range(5): ts[t, pl.ds(m2 * P + 64*h, 64), :] = y[t]
            return f
        return [z0, zab(1), zab(2), dinv(0), dinv(1)]
    def st5(b):
        def f():
            for t in range(5):
                for a in range(8):
                    z = ts[t, pl.ds(8*b + a, 16, stride=P), :]
                    if '5' in PACE and anc['z'] is not None: z = z + jnp.concatenate([zvec()] * 2, axis=0)
                    outa_v[pl.ds(b*128 + 16*a, 16), 128*t:128*t+128] = z.astype(BF)
            out_a(b).start()
        return f

    def spread(items, lo, hi, ex):
        n = hi - lo
        for k, f in enumerate(items): ex[lo + k * n // max(len(items), 1)].append(f)
    def chunk(items, its):
        out = {b: [] for b in its}
        for k, f in enumerate(items): out[its[k * len(its) // len(items)]].append(f)
        return out
    def mix(a_, b_):
        pos = [((k + 0.5) / len(a_), 0, k) for k in range(len(a_))] + [((k + 0.5) / len(b_), 1, k) for k in range(len(b_))]
        return [(a_, b_)[w][k] for _, w, k in sorted(pos)]
    rng = lambda name, d: [int(x) for x in d.split(',')]
    def bar():
        pl.semaphore_signal(sem_bar); pl.semaphore_wait(sem_bar)
    plan1 = {b: [] for b in range(NB)}
    def add(plan, d):
        for b, v in d.items(): plan[b] += v
    add(plan1, chunk([f for k in range(8) for f in st1(k)], rng("S1", "4,5")))
    add(plan1, chunk([f for k in range(8, 16) for f in st1(k)], rng("S1b", "6")))
    add(plan1, chunk([f for k in range(16) for f in st2(k)], rng("S2", "7,8,9")))
    add(plan1, chunk([wprep(k) for k in range(16)], rng("SW", "10")))
    lst3 = []
    for rr in range(8):
        lst3 += st3_items(rr)
        if rr % 2: lst3 += st3_fin(rr)
    S3A, S3B = rng("S3", "10,11,12,13,14,15"), [x for x in rng("S3B", "-1") if x >= 0]
    d3 = chunk(lst3, [("I", x) for x in S3A] + [("II", x) for x in S3B])
    add(plan1, {k[1]: v for k, v in d3.items() if k[0] == "I"})
    p0, p1_ = proj_items(0), proj_items(1)
    with scope("pro_wait0"):
        cp_x(0).wait(); cp_x(1).wait(); cp_wg(1).wait()
    cp_wg(2).start(); cp_x(2).start(priority=1); cp_x(3).start(priority=1); cp_a(0).start(priority=1)
    for n in WORDER[0:5]:
        for f in p0[n] + p1_[n]: f()
    with scope("pro_w1"):
        cp_wg(0).wait()
    for n in WORDER[5:10]:
        for f in p0[n] + p1_[n]: f()
    with scope("pro_w2"):
        cp_wg(2).wait(); cp_x(2).wait()
    cp_a(1).start(priority=1)
    for n in WORDER[10:15]:
        for f in p0[n] + p1_[n]: f()
    W1 = {4: [lambda: cp_x(3), lambda: cp_a(0)],
          6: [lambda: cp_a(1), lambda: cp_dm, lambda: cp_ft, lambda: cp_x(4)], 10: [lambda: cp_wr, lambda: cp_wi, lambda: cp_x(5), lambda: cp_wo, lambda: cp_hs]}
    S1_ = {2: [lambda: cp_dm, lambda: cp_ft, lambda: cp_x(4)], 4: [lambda: cp_wr, lambda: cp_wi, lambda: cp_x(5)], 6: [lambda: cp_wo, lambda: cp_hs]}
    for b in range(2, NB):
        with scope(f'w1_{b:02d}'):
            for f in W1.get(b, []): f().wait()
        for f in S1_.get(b, []): f().start(priority=1)
        if b in rng("BAR1", "-1"): bar()
        pi = proj_items(b)
        for f in mix([g for n in WORDER for g in pi[n]], plan1[b]): f()
    plan2 = {b: [] for b in range(NB)}
    add(plan2, {k[1]: v for k, v in d3.items() if k[0] == "II"})
    add(plan2, chunk([f for k in range(16) for f in st4(k)], rng("S4", "0,1,2,3,4,5,6,7")))
    add(plan2, chunk([st5(k) for k in range(16)], rng("S5", "9,10")))
    EX = {}
    for b in range(NB):
        ex = [[] for _ in range(NT_)]
        spread(plan2[b], 0, NT_, ex)
        if b > 0: spread(outproj_items(b - 1), LA + LB + HP, LA + LB + HP + E("ES", 16), ex)
        EX[b] = ex
    def marks(b):
        if b in rng("BAR2", "0"): bar()
    attn_flow(list(range(NB)), EX, marks)
    with scope('epi'):
        for f in outproj_items(NB - 1): f()
    with scope('epi_wait'):
        for b in range(NB): out_b(b).wait()
        for b in range(NB): out_a(b).wait()

_DM, _FT, _HS = a_consts3()

@jax.jit
def pallas_concat_heads__spectral_gfnet__sliding_block__prompt_kernel(A_x, A_w_r, A_w_i, B_x, B_wqkv, B_wo):
    anyspec = pl.BlockSpec(memory_space=pl.ANY)
    V = pltpu.VMEM
    return pl.pallas_call(
        kernel,
        out_shape=jax.ShapeDtypeStruct((1, S, 2*D), BF),
        in_specs=[anyspec]*9, out_specs=anyspec,
        scratch_shapes=[
            V((S, D), BF), V((DF, S), BF), V((DF, S), BF), V((16, 128, 256), BF), V((16, 256, 128), BF), V((6, 256, 256), BF),
            V((5, 16*P, 128), F32), V((6, 16, 128, 128), F32), V((6, 16, 64, 128), U32), V((2, 16, 328, 128), F32), V((S, D), BF),
            V((S, D), BF), V((D, 3*D), BF), V((D, D), BF),
            V((8, S//2, 128), U32), V((D//2, S), U32), V((D, S), F32), V((NB, D, 128), F32), V((S, D), BF),
            V((2, 5, 64, 128), U32), V((2, 128, D), BF),
            pltpu.SemaphoreType.DMA((16,)), pltpu.SemaphoreType.DMA((6,)), pltpu.SemaphoreType.DMA((7,)),
            pltpu.SemaphoreType.DMA(()), pltpu.SemaphoreType.DMA(()), pltpu.SemaphoreType.REGULAR,
        ],
        compiler_params=pltpu.CompilerParams(vmem_limit_bytes=120*2**20),
        name="kG",
    )(A_x, A_w_r.T, A_w_i.T, B_x, B_wqkv, B_wo, jnp.asarray(_FT), jnp.asarray(_HS), jnp.asarray(_DM))
```

```python
import contextlib
def scope(n): return contextlib.nullcontext()
import numpy as np
import ml_dtypes
import jax
import jax.numpy as jnp
from jax import lax
from jax.experimental import pallas as pl
from jax.experimental.pallas import tpu as pltpu
BFn = ml_dtypes.bfloat16

S, D, H, DH = 2048, 640, 32, 20
DF = 321
BQ = 128
NB = S // BQ
BF, F32, U32 = jnp.bfloat16, jnp.float32, jnp.uint32
QSCALE = float(DH ** -0.5 * np.log2(np.e))
NEG = -1e30
P = 132
c1, c2, s1, s2 = (float(np.cos(2*np.pi/5)), float(np.cos(4*np.pi/5)), float(np.sin(2*np.pi/5)), float(np.sin(4*np.pi/5)))
E = lambda k, d: d
HP = E("HP", 2); LA = E("LA", 1); LB = E("LB", 3)
NQ = 128 // HP; NP = NQ // 16; NMID = (256 - NQ) // 16; NGRP = 2*NP + NMID
NT = (((1,), (1,)), ((), ()))
def freq_lanes(c):
    l = np.arange(128)
    return np.where(l < 64, 5*l + c, 5*(l-64) + (5-c))
def d_mats():
    d1 = np.arange(128)[:, None].astype(np.float64)
    out = []
    for c in (1, 2):
        f = freq_lanes(c)[None, :].astype(np.float64)
        sg = np.where(np.arange(128)[None, :] < 64, 1.0, -1.0)
        C = np.cos(2*np.pi*f*d1/D); Sn = -np.sin(2*np.pi*f*d1/D)
        M = np.zeros((256, 256))
        M[:128, :128] = C; M[128:, :128] = -sg*Sn; M[:128, 128:] = Sn; M[128:, 128:] = sg*C
        out.append(M)
    l = np.arange(128)[None, :]
    fre = 5.0*l; fim = 5.0*(l-64)
    M0 = np.where(l <= 64, np.cos(2*np.pi*fre*d1/D), -np.sin(2*np.pi*fim*d1/D))
    MA, MB = out
    IA = MA.T*2.0/D; IB = MB.T*2.0/D
    cf = np.where((l == 0) | (l == 64), 1.0, 2.0)
    I0 = (M0*cf).T / D
    return M0, MA, MB, I0, IA, IB
def s_mats():
    k1 = np.arange(128)[:, None]; n1 = np.arange(128)[None, :]
    F = np.zeros((16, 256, 128)); Hh = np.zeros((16, 256, 128))
    for n2 in range(16):
        ph = 2*np.pi*((k1*(16*n1+n2)) % S)/S
        F[n2, :128] = np.cos(ph); F[n2, 128:] = -np.sin(ph)
        Hh[n2, :128] = np.cos(ph).T/S; Hh[n2, 128:] = np.sin(ph).T/S
    return F, Hh
def a_consts2():
    M0, MA, MB, I0, IA, IB = d_mats()
    dm = np.zeros((6, 256, 256), np.float32)
    dm[0, :128, :128] = M0.T; dm[1] = MA.T; dm[2] = MB.T
    dm[3, :128, :128] = I0; dm[4] = IA; dm[5] = IB
    F, Hh = s_mats()
    FT = np.concatenate([F[:, :128].transpose(0, 2, 1), F[:, 128:].transpose(0, 2, 1)], axis=2)
    return dm.astype(BFn), FT.astype(np.float32).astype(BFn), Hh.astype(np.float32).astype(BFn)

def a_consts3():
    dm, FT, HS = a_consts2()
    perm = np.arange(128).reshape(8, 2, 8).transpose(0, 2, 1).reshape(128)
    dm = dm.copy()
    dm[3, :128] = dm[3, :128][perm]
    for k in (4, 5):
        dm[k, :128] = dm[k, :128][perm]
        dm[k, 128:] = dm[k, 128:][perm]
    return dm, FT, HS

def cmul_const(ar, ai, w):
    wr_, wi_ = round(w.real, 12), round(w.imag, 12)
    if wi_ == 0 and wr_ == 1: return ar, ai
    if wi_ == 0 and wr_ == -1: return -ar, -ai
    if wr_ == 0 and wi_ == 1: return -ai, ar
    if wr_ == 0 and wi_ == -1: return ai, -ar
    if abs(abs(wr_) - abs(wi_)) < 1e-12:
        k = abs(wr_); sr, si = np.sign(wr_), np.sign(wi_)
        if sr > 0 and si > 0: return (ar - ai)*k, (ar + ai)*k
        if sr > 0 and si < 0: return (ar + ai)*k, (ai - ar)*k
        if sr < 0 and si > 0: return (ar + ai)*(-k), (ar - ai)*k
        return (ai - ar)*k, (ar + ai)*(-k)
    return ar*wr_ - ai*wi_, ar*wi_ + ai*wr_

def dft4(x, sign):
    (ar, ai), (br, bi), (cr, ci), (dr, di) = x
    t0r, t0i = ar + cr, ai + ci
    t1r, t1i = ar - cr, ai - ci
    t2r, t2i = br + dr, bi + di
    t3r, t3i = br - dr, bi - di
    if sign < 0:
        x1 = (t1r + t3i, t1i - t3r); x3 = (t1r - t3i, t1i + t3r)
    else:
        x1 = (t1r - t3i, t1i + t3r); x3 = (t1r + t3i, t1i - t3r)
    return [(t0r + t2r, t0i + t2i), x1, (t0r - t2r, t0i - t2i), x3]

def dft16(x, sign):
    cols = []
    for n2 in range(4):
        y = dft4([x[4*n1 + n2] for n1 in range(4)], sign)
        y = [cmul_const(y[k1][0], y[k1][1], np.exp(sign*2j*np.pi*n2*k1/16)) for k1 in range(4)]
        cols.append(y)
    out = [None]*16
    for k1 in range(4):
        z = dft4([cols[n2][k1] for n2 in range(4)], sign)
        for k2 in range(4): out[k1 + 4*k2] = z[k2]
    return out


def ntdot(a, b): return lax.dot_general(a, b, NT, preferred_element_type=F32)
def dot(a, b): return jnp.dot(a, b, preferred_element_type=F32)
def bc(x): return pltpu.bitcast(x, BF)
def pk2(a, b): return pltpu.bitcast(jnp.concatenate([a, b], axis=0).astype(BF), U32)
def tree(xs, f):
    xs = list(xs)
    while len(xs) > 1:
        xs = [f(xs[k], xs[k+1]) if k + 1 < len(xs) else xs[k] for k in range(0, len(xs), 2)]
    return xs[0]
def split_pieces(groups, firsts, lasts, flip):
    units = [[f, l] for f, l in zip(firsts, lasts) if f in groups and l in groups]
    paired = {g for u in units for g in u}
    singles = [g for g in groups if g not in paired]
    n = len(groups)
    sizes = [n // 4] * 4
    order = [2, 3, 0, 1] if flip else [0, 1, 2, 3]
    for k in range(n - sum(sizes)): sizes[order[k]] += 1
    pcs = [[] for _ in range(4)]
    k = 0
    for u in units:
        tries = 0
        while len(pcs[k]) + 2 > sizes[k] and tries < 4: k = (k + 1) % 4; tries += 1
        if tries == 4: singles += u; continue
        pcs[k] += u; k = (k + 1) % 4
    for k in range(4):
        while len(pcs[k]) < sizes[k]: pcs[k].append(singles.pop(0))
    assert not singles
    return [p for p in pcs if p]

def kernel(ax_hbm, wr_hbm, wi_hbm, bx_hbm, wqkv_hbm, wo_hbm, ft_hbm, hs_hbm, dm_hbm, out_hbm,
           ax_v, wr_v, wi_v, ft_v, hs_v, dm_v, ts, g_s, u_s, wf, outa_v,
           bx_v, wqkv_v, wo_v, kg_s, qT_s, vT_s, oT_s, outb_v, kt_s, ol_s,
           sem_w, sem_x, sem_a, sem_outa, sem_outb, sem_bar):
    WORDER = [5, 6, 7, 8, 9, 0, 1, 2, 3, 4, 10, 11, 12, 13, 14]
    def cp_w(n): return pltpu.make_async_copy(wqkv_hbm.at[:, pl.ds(128*n, 128)], wqkv_v.at[:, pl.ds(128*n, 128)], sem_w.at[n])
    def cp_wg(g): return pltpu.make_async_copy(wqkv_hbm.at[:, pl.ds(640*g, 640)], wqkv_v.at[:, pl.ds(640*g, 640)], sem_w.at[g])
    XCH = [(0, 128), (128, 256), (256, 512), (512, 1024), (1024, 1536), (1536, 2048)]
    def cp_x(c):
        lo, hi = XCH[c]
        return pltpu.make_async_copy(bx_hbm.at[0, pl.ds(lo, hi - lo), :], bx_v.at[pl.ds(lo, hi - lo), :], sem_x.at[c])
    ACH = [(0, 1024), (1024, 2048)]
    def cp_a(c):
        lo, hi = ACH[c]
        return pltpu.make_async_copy(ax_hbm.at[0, pl.ds(lo, hi - lo), :], ax_v.at[pl.ds(lo, hi - lo), :], sem_a.at[c])
    cp_wr = pltpu.make_async_copy(wr_hbm, wr_v, sem_a.at[2])
    cp_wi = pltpu.make_async_copy(wi_hbm, wi_v, sem_a.at[3])
    cp_ft = pltpu.make_async_copy(ft_hbm, ft_v, sem_a.at[4])
    cp_hs = pltpu.make_async_copy(hs_hbm, hs_v, sem_a.at[5])
    cp_dm = pltpu.make_async_copy(dm_hbm, dm_v, sem_a.at[6])
    cp_wo = pltpu.make_async_copy(wo_hbm, wo_v, sem_w.at[15])
    cp_x(0).start(); cp_x(1).start()
    cp_wg(1).start()
    cp_wg(0).start()

    row8 = lax.broadcasted_iota(jnp.int32, (8, 128), 0)
    col8 = lax.broadcasted_iota(jnp.int32, (8, 128), 1)
    col64 = lax.broadcasted_iota(jnp.int32, (64, 128), 1)
    DQ = row8 - (col8 & (NQ - 1))
    lo4 = row8 < 4
    part = col8 >> int(np.log2(NQ)) if HP > 1 else col8 * 0
    bits = [((part >> k) & 1) == 1 for k in range(int(np.log2(HP)))]
    zero_u = jnp.zeros((8, 128), U32)

    anc = {'z': None}
    PACE = "13w"
    def zvec():
        k = min(anc['k'], 15); anc['k'] += E("PSTEP", 3)
        y = anc['src'][8*k:8*k+8]
        return y - y
    def pace(x, st):
        return x if (anc['z'] is None or st not in PACE) else x + zvec()
    def pace_u(x, n, st):
        if anc['z'] is None or st not in PACE: return x
        z = pltpu.bitcast(zvec(), U32)
        return jnp.concatenate([x[0:8] | z, x[8:n]], axis=0)
    def proj_items(b):
        r0 = b * BQ; u0 = b * 64
        def mm(n):
            y = dot(bx_v[pl.ds(r0, BQ), :], wqkv_v[:, 128*n:128*n+128])
            if PACE: anc['src'] = y; anc['k'] = 0; anc['z'] = True
            return y
        def qtile(t):
            def f():
                q = (mm(t) * QSCALE).astype(BF)
                qT_s[64*t:64*t+64, pl.ds(r0, BQ)] = pltpu.bitcast(q.T, U32)
            return f
        def vtile(t):
            def f():
                v = mm(10 + t)
                vT_s[128*t:128*t+128, pl.ds(r0, BQ)] = v.astype(BF).T.astype(F32)
            return f
        def ktile(t):
            def f(): kt_s[b % 2, t] = pltpu.bitcast(mm(5 + t).astype(BF), U32)
            return f
        def kgrp(j):
            def f():
                t0, off = divmod(80 * j, 128)
                a = kt_s[b % 2, t0]
                if off > 0: a = pltpu.roll(a, 128 - off, 1)
                if off + 80 > 128:
                    a = jnp.where(col64 < 128 - off, a, pltpu.roll(kt_s[b % 2, t0 + 1], 128 - off, 1))
                kg_s[j, pl.ds(u0, 64), :] = jnp.where(col64 < 80, a, U32(0))
            return f
        by_tile = {5: [ktile(0), kgrp(0)], 6: [ktile(1), kgrp(1), kgrp(2)], 7: [ktile(2), kgrp(3)], 8: [ktile(3), kgrp(4), kgrp(5)], 9: [ktile(4), kgrp(6), kgrp(7)]}
        for t in range(5):
            by_tile[t] = [qtile(t)]; by_tile[10 + t] = [vtile(t)]
        return by_tile

    def outproj_items(b):
        r0 = b * BQ
        def tr(t):
            def f(): ol_s[b % 2, :, 128*t:128*t+128] = oT_s[b, 128*t:128*t+128, :].astype(BF).T
            return f
        def mm(n):
            def f(): outb_v[pl.ds(r0, BQ), 128*n:128*n+128] = dot(ol_s[b % 2], wo_v[:, 128*n:128*n+128]).astype(BF)
            return f
        def dma():
            out_b(b).start()
        return [tr(t) for t in range(5)] + [mm(n) for n in range(5)] + [dma]
    def out_b(b):
        return pltpu.make_async_copy(outb_v.at[pl.ds(b*BQ, BQ), :], out_hbm.at[0, pl.ds(b*BQ, BQ), pl.ds(D, D)], sem_outb)
    def out_a(b):
        return pltpu.make_async_copy(outa_v.at[pl.ds(b*BQ, BQ), :], out_hbm.at[0, pl.ds(b*BQ, BQ), pl.ds(0, D)], sem_outa)

    def attn_ctx(b):
        q0 = b * 128
        def make_R(j, heads):
            R = {}
            for ii, i in enumerate(heads):
                lo, hi = 10*i, 10*i + 10
                for t in range(lo//8, (hi-1)//8 + 1):
                    q = qT_s[pl.ds(40*j + 8*t, 8), pl.ds(q0, 128)]
                    if ii > 0: q = pltpu.roll(q, NQ*ii, 1)
                    rlo, rhi = max(lo - 8*t, 0), min(hi - 8*t, 8)
                    R.setdefault(t, []).append((ii, q, rlo, rhi))
            return R
        def make_qm(R, a):
            out = []
            for t in range(5):
                if t not in R: out.append(zero_u); continue
                v = zero_u
                for (ii, q, rlo, rhi) in R[t]:
                    full = (rlo == 0 and rhi == 8)
                    msk = None if full else ((row8 >= rlo) & (row8 < rhi))
                    if HP > 1:
                        pm = part == (ii + a) % HP
                        msk = pm if msk is None else (msk & pm)
                    v = q if msk is None else jnp.where(msk, q, v)
                out.append(v)
            return bc(jnp.concatenate(out, axis=0))
        def key0(a): return q0 - 256 + NQ * a
        def valid(a):
            return [g for g in range(NGRP) if key0(a) + 16*g >= 0]
        def qk_tile(j, a, R):
            qm = make_qm(R, a)
            base = (key0(a)) // 2
            def rows(ids): return bc(jnp.concatenate([kg_s[j, pl.ds(base + 8*g, 8), :] for g in ids], axis=0))[:, 0:80]
            vals = {}
            for ids in split_pieces(valid(a), list(range(NP)), list(range(NP + NMID, NGRP)), a % 2):
                s = dot(rows(ids), qm)
                for n, g in enumerate(ids):
                    vals[g] = (s[16*n:16*n+8], s[16*n+8:16*n+16])
            cs = []
            for r in range(2*NP):
                g, hh = divmod(r, 2)
                fst = vals[g][hh] if g in vals else NEG
                cs.append(jnp.where(DQ > -8*r, fst, vals[NP + NMID + g][hh]))
            mid = {g: vals[g] for g in range(NP, NP + NMID) if g in vals}
            return cs, mid, [g in vals for g in range(NP)]
        def sm_tile(cs, mid, has_first):
            allv = cs + [x for g in mid for x in mid[g]]
            m8 = tree(allv, jnp.maximum)
            if 'a' in PACE: anc['src'] = jnp.concatenate([m8] * 16, axis=0); anc['k'] = 0; anc['z'] = True
            m = jnp.max(m8, axis=0, keepdims=True)
            pc = [jnp.exp2(c - m) for c in cs]
            Pg = {}
            for g in range(NP):
                if has_first[g]:
                    p0 = [jnp.where(DQ > -8*(2*g + hh), pc[2*g + hh], 0.0) for hh in range(2)]
                    Pg[g] = pk2(p0[0], p0[1])
                    Pg[NP + NMID + g] = pk2(pc[2*g] - p0[0], pc[2*g + 1] - p0[1])
                else:
                    Pg[NP + NMID + g] = pk2(pc[2*g], pc[2*g + 1])
            for g in mid:
                Pg[g] = pk2(jnp.exp2(mid[g][0] - m), jnp.exp2(mid[g][1] - m))
            return Pg
        kt_lo = max(0, (256 - q0) // 128)
        def merge(Ps):
            out = [[] for _ in range(HP)]
            for gam in range(8 * kt_lo, 24):
                s = [Ps[a].get(gam - NP*a) if 0 <= gam - NP*a < NGRP else None for a in range(HP)]
                def sel(mask, x, y):
                    if x is None and y is None: return None
                    return jnp.where(mask, zero_u if x is None else x, zero_u if y is None else y)
                w = s
                for k, bit in enumerate(bits):
                    w = [sel(bit, w[(n + (1 << k)) % HP], w[n]) for n in range(HP)]
                if HP == 1: w = s
                for i in range(HP):
                    v = w[(-i) % HP]
                    out[i].append(zero_u if v is None else v)
            return [jnp.concatenate(o, axis=0) for o in out]
        def pv(h, ii, p):
            w0 = (20*h)//8*8; off = 20*h - w0
            nk = 384 - 128 * kt_lo
            vt = vT_s[pl.ds(w0, 24), pl.ds(q0 - 256 + 128*kt_lo, nk)]
            grow = 23 if off == 0 else 0
            blk = grow // 8
            parts = [vt[8*t:8*t+8] for t in range(3)]
            parts[blk] = jnp.where(lax.broadcasted_iota(jnp.int32, (8, nk), 0) == grow % 8, 1.0, parts[blk])
            o = dot(jnp.concatenate(parts, axis=0), bc(p))
            o = o * (1.0 / o[grow:grow+1])
            if ii > 0: o = pltpu.roll(o, 128 - NQ*ii, 1)
            return o
        def flush(j, outs):
            o0, o1, o2, o3 = outs
            oT = [o0[0:16], jnp.where(lo4, o0[16:24], o1[0:8]), o1[8:24], o2[0:16], jnp.where(lo4, o2[16:24], o3[0:8]), o3[8:24]]
            oT_s[b, pl.ds(80*j, 80), :] = jnp.concatenate(oT, axis=0)
        return make_R, qk_tile, sm_tile, merge, pv, flush
    sets = [(j, list(range(i0, i0+HP))) for j in range(8) for i0 in range(0, 4, HP)]
    NT_ = len(sets) * HP
    def attn_flow(blocks, extras, marks=None):
        ctx = {b: attn_ctx(b) for b in blocks}
        tiles = [(b, t) for b in blocks for t in range(NT_)]
        n = len(tiles)
        st = {}; ps = {}; R = {}; mg = {}; outs = {}
        for g in range(n + LA + LB + HP):
            if g < n:
                b, t = tiles[g]
                if t == 0 and marks: marks(b)
                si, a = divmod(t, HP)
                if a == 0: R[(b, si)] = ctx[b][0](*sets[si])
                st[g] = ctx[b][1](sets[si][0], a, R[(b, si)])
                if a == HP - 1: R.pop((b, si))
                for f in extras[b][t]: f()
            u = g - LA
            if 0 <= u < n: ps[u] = ctx[tiles[u][0]][2](*st.pop(u))
            v = g - LB - (HP - 1)
            if 0 <= v < n:
                b, t = tiles[v]
                si, ii = divmod(t, HP)
                j, heads = sets[si]
                if ii == 0: mg[v] = ctx[b][3]([ps.pop(v + a) for a in range(HP)])
                h = 4*j + heads[ii]
                outs[(b, h)] = ctx[b][4](h, ii, mg[v - ii][ii])
                if ii == HP - 1: mg.pop(v - ii)
                if h % 4 == 3: ctx[b][5](j, [outs.pop((b, 4*j + k)) for k in range(4)])

    def st1(b):
        def piece(a):
            def f():
                r0 = b * 128 + 16 * a
                xt = [ax_v[pl.ds(r0, 16), 128*t:128*t+128].astype(F32) for t in range(5)]
                if '1' in PACE and anc['z'] is not None:
                    z2 = jnp.concatenate([zvec()] * 2, axis=0)
                    xt[1] = xt[1] + z2; xt[2] = xt[2] + z2
                b_, c_, d_, e_ = xt[1] + xt[4], xt[2] + xt[3], xt[1] - xt[4], xt[2] - xt[3]
                T = [xt[0] + b_ + c_, xt[0] + c1*b_ + c2*c_, -s1*d_ - s2*e_, xt[0] + c2*b_ + c1*c_, s1*e_ - s2*d_]
                for t in range(5):
                    ts[t, pl.ds(8*b + a, 16, stride=P), :] = T[t]
            return f
        return [piece(a) for a in range(8)]
    def wprep(k2):
        def f():
            for a, src in enumerate((wr_v, wi_v)):
                for r in range(0, 320, 32):
                    w = src[r:r+32, pl.ds(128*k2, 128)].astype(F32)
                    if 'w' in PACE and anc['z'] is not None: w = w + jnp.concatenate([zvec()] * 4, axis=0)
                    wf[a, k2, r:r+32, :] = w
                wf[a, k2, 320:321, :] = src[320:321, pl.ds(128*k2, 128)].astype(F32)
        return f
    def st2(n2):
        base = n2 * P
        def ldT(t): return ts[t, pl.ds(base, 128), :].astype(BF)
        V2 = E("V2", 0)
        def whole():
            T = [ldT(t) for t in range(5)]
            Z0 = ntdot(dm_v[0, 0:128, 0:128], T[0])
            ZA = ntdot(dm_v[1], jnp.concatenate(T[1:3], axis=1))
            ZB = ntdot(dm_v[2], jnp.concatenate(T[3:5], axis=1))
            ZT = jnp.concatenate([Z0, ZA, ZB], axis=0).astype(BF)
            PT = dot(ZT, ft_v[n2])
            g_s[0, n2] = PT[0:128, 0:128]; g_s[1, n2] = PT[0:128, 128:256]
            g_s[2, n2] = PT[128:256, 0:128] - PT[256:384, 128:256]; g_s[3, n2] = PT[128:256, 128:256] + PT[256:384, 0:128]
            g_s[4, n2] = PT[384:512, 0:128] - PT[512:640, 128:256]; g_s[5, n2] = PT[384:512, 128:256] + PT[512:640, 0:128]
        def g0():
            z = ntdot(dm_v[0, 0:128, 0:128], ldT(0)).astype(BF)
            PT = dot(z, ft_v[n2])
            g_s[0, n2] = PT[:, 0:128]; g_s[1, n2] = PT[:, 128:256]
        def gab(g):
            def f():
                Z = ntdot(dm_v[g], jnp.concatenate([ldT(2*g - 1), ldT(2*g)], axis=1)).astype(BF)
                PT = dot(Z, ft_v[n2])
                g_s[2*g, n2] = PT[0:128, 0:128] - PT[128:256, 128:256]
                g_s[2*g + 1, n2] = PT[0:128, 128:256] + PT[128:256, 0:128]
            return f
        return [whole] if V2 == 0 else [g0, gab(1), gab(2)]
    def ldc(g, pos, r0): return (g_s[2*g, pos, pl.ds(r0, 8), :], g_s[2*g+1, pos, pl.ds(r0, 8), :])
    def stc(g, pos, r0, v):
        g_s[2*g, pos, pl.ds(r0, 8), :] = v[0]
        g_s[2*g+1, pos, pl.ds(r0, 8), :] = v[1]
    def tw(v, n, sign): return cmul_const(v[0], v[1], np.exp(sign * 2j * np.pi * n / 16))
    def p1(g, r0):
        def one(n2):
            def f():
                xs = [ldc(g, 4*n1 + n2, r0) for n1 in range(4)]
                xs[0] = (pace(xs[0][0], '3'), xs[0][1])
                y = dft4(xs, -1)
                for k1 in range(4): stc(g, 4*k1 + n2, r0, tw(y[k1], n2*k1, -1))
            return f
        return [one(n2) for n2 in range(4)]
    def mulw(x, k2, wrow, special=None):
        wr = wf[0, k2, pl.ds(wrow, 8, stride=5), :]
        wi = wf[1, k2, pl.ds(wrow, 8, stride=5), :]
        if special is not None:
            wr = jnp.where(special, wf[0, k2, 320:321, :], wr); wi = jnp.where(special, wf[1, k2, 320:321, :], wi)
        return (x[0]*wr - x[1]*wi, x[0]*wi + x[1]*wr)
    def inv1(g, r0, k1, Y):
        u = dft4(Y, +1)
        for j1 in range(4): stc(g, 4*k1 + j1, r0, tw(u[j1], k1*j1, +1))
    def p2ab(g, rr, half):
        c = ((1, 4), (2, 3))[g-1][half]
        r0 = rr*8 + 64*half
        def one(k1):
            def f():
                xs = [ldc(g, 4*k1 + n2, r0) for n2 in range(4)]
                xs[0] = (pace(xs[0][0], '3'), xs[0][1])
                X = dft4(xs, -1)
                inv1(g, r0, k1, [mulw(X[k2], k1 + 4*k2, 40*rr + c) for k2 in range(4)])
            return f
        return [one(k1) for k1 in range(4)]
    def p2g0(rr):
        r0, r1 = rr*8, rr*8 + 64
        def one(k1):
            def f():
                xa = [ldc(0, 4*k1 + n2, r0) for n2 in range(4)]; xb = [ldc(0, 4*k1 + n2, r1) for n2 in range(4)]
                xa[0] = (pace(xa[0][0], '3'), xa[0][1]); xb[0] = (pace(xb[0][0], '3'), xb[0][1])
                Xa = dft4(xa, -1); Xb = dft4(xb, -1)
                Ya, Yb = [], []
                for k2 in range(4):
                    ar, ai = Xa[k2]; br, bi = Xb[k2]
                    if rr == 0:
                        keep = row8 == 0
                        A2 = (jnp.where(keep, ar, ar - bi), jnp.where(keep, ai, ai + br))
                        B2 = (jnp.where(keep, br, br + ai), jnp.where(keep, bi, bi - ar))
                    else:
                        A2 = (ar - bi, ai + br); B2 = (br + ai, bi - ar)
                    Ya.append(mulw(A2, k1 + 4*k2, 40*rr))
                    Yb.append(mulw(B2, k1 + 4*k2, 40*rr, special=(row8 == 0) if rr == 0 else None))
                inv1(0, r0, k1, Ya); inv1(0, r1, k1, Yb)
            return f
        return [one(k1) for k1 in range(4)]
    def p3(g, rp):
        def one(j1):
            def f():
                xa = [ldc(g, 4*k1 + j1, 16*rp) for k1 in range(4)]; xb = [ldc(g, 4*k1 + j1, 16*rp + 8) for k1 in range(4)]
                xa[0] = (pace(xa[0][0], '3'), xa[0][1]); xb[0] = (pace(xb[0][0], '3'), xb[0][1])
                ua = dft4(xa, +1); ub = dft4(xb, +1)
                for j2 in range(4):
                    m2 = j1 + 4*j2
                    u_s[2*g, m2, pl.ds(8*rp, 8), :] = pk2(ua[j2][0], ub[j2][0])
                    u_s[2*g+1, m2, pl.ds(8*rp, 8), :] = pk2(ua[j2][1], ub[j2][1])
            return f
        return [one(j1) for j1 in range(4)]
    def st3_items(rr):
        it = []
        for g in range(3):
            it += p1(g, 8*rr) + p1(g, 8*rr + 64)
        it += p2ab(1, rr, 0) + p2ab(1, rr, 1) + p2g0(rr) + p2ab(2, rr, 0) + p2ab(2, rr, 1)
        return it
    def st3_fin(rr):
        return [f for g in range(3) for rp in (rr//2, 4 + rr//2) for f in p3(g, rp)]
    def st4(m2):
        zz = {}
        def hr(): return hs_v[m2, 0:128, :]
        def hi(): return hs_v[m2, 128:256, :]
        def z0():
            zz[0] = (ntdot(hr(), bc(u_s[0, m2])) - ntdot(hi(), bc(u_s[1, m2]))).astype(BF)
        def zab(g):
            def f():
                ur, ui = bc(u_s[2*g, m2]), bc(u_s[2*g + 1, m2])
                zr = ntdot(hr(), ur) - ntdot(hi(), ui)
                zi = ntdot(hi(), ur) + ntdot(hr(), ui)
                zz[g] = jnp.concatenate([zr, zi], axis=1).astype(BF)
            return f
        def dinv(h):
            def f():
                rows = slice(64*h, 64*h + 64)
                V0 = dot(zz[0][rows], dm_v[3, 0:128, 0:128])
                U1 = dot(zz[1][rows], dm_v[4]); U2 = dot(zz[2][rows], dm_v[5])
                U1r, U1i, U2r, U2i = U1[:, :128], U1[:, 128:], U2[:, :128], U2[:, 128:]
                p = V0 + c1*U1r + c2*U2r; q = s1*U1i + s2*U2i
                pp = V0 + c2*U1r + c1*U2r; qq = s2*U1i - s1*U2i
                y = [V0 + U1r + U2r, p - q, pp - qq, pp + qq, p + q]
                for t in range(5): ts[t, pl.ds(m2 * P + 64*h, 64), :] = y[t]
            return f
        return [z0, zab(1), zab(2), dinv(0), dinv(1)]
    def st5(b):
        def f():
            for t in range(5):
                for a in range(8):
                    z = ts[t, pl.ds(8*b + a, 16, stride=P), :]
                    if '5' in PACE and anc['z'] is not None: z = z + jnp.concatenate([zvec()] * 2, axis=0)
                    outa_v[pl.ds(b*128 + 16*a, 16), 128*t:128*t+128] = z.astype(BF)
            out_a(b).start()
        return f

    def spread(items, lo, hi, ex):
        n = hi - lo
        for k, f in enumerate(items): ex[lo + k * n // max(len(items), 1)].append(f)
    def chunk(items, its):
        out = {b: [] for b in its}
        for k, f in enumerate(items): out[its[k * len(its) // len(items)]].append(f)
        return out
    def mix(a_, b_):
        pos = [((k + 0.5) / len(a_), 0, k) for k in range(len(a_))] + [((k + 0.5) / len(b_), 1, k) for k in range(len(b_))]
        return [(a_, b_)[w][k] for _, w, k in sorted(pos)]
    rng = lambda name, d: [int(x) for x in d.split(',')]
    def bar():
        pl.semaphore_signal(sem_bar); pl.semaphore_wait(sem_bar)
    plan1 = {b: [] for b in range(NB)}
    def add(plan, d):
        for b, v in d.items(): plan[b] += v
    add(plan1, chunk([f for k in range(8) for f in st1(k)], rng("S1", "4,5")))
    add(plan1, chunk([f for k in range(8, 16) for f in st1(k)], rng("S1b", "6")))
    add(plan1, chunk([f for k in range(16) for f in st2(k)], rng("S2", "7,8,9")))
    add(plan1, chunk([wprep(k) for k in range(16)], rng("SW", "10")))
    lst3 = []
    for rr in range(8):
        lst3 += st3_items(rr)
        if rr % 2: lst3 += st3_fin(rr)
    S3A, S3B = rng("S3", "10,11,12,13,14,15"), [x for x in rng("S3B", "-1") if x >= 0]
    d3 = chunk(lst3, [("I", x) for x in S3A] + [("II", x) for x in S3B])
    add(plan1, {k[1]: v for k, v in d3.items() if k[0] == "I"})
    p0, p1_ = proj_items(0), proj_items(1)
    with scope("pro_wait0"):
        cp_x(0).wait(); cp_x(1).wait(); cp_wg(1).wait()
    cp_wg(2).start(); cp_x(2).start(priority=1); cp_x(3).start(priority=1); cp_a(0).start(priority=1)
    for n in WORDER[0:5]:
        for f in p0[n] + p1_[n]: f()
    with scope("pro_w1"):
        cp_wg(0).wait()
    for n in WORDER[5:10]:
        for f in p0[n] + p1_[n]: f()
    with scope("pro_w2"):
        cp_wg(2).wait(); cp_x(2).wait()
    cp_a(1).start(priority=1)
    for n in WORDER[10:15]:
        for f in p0[n] + p1_[n]: f()
    W1 = {4: [lambda: cp_x(3), lambda: cp_a(0)],
          6: [lambda: cp_a(1), lambda: cp_dm, lambda: cp_ft, lambda: cp_x(4)], 10: [lambda: cp_wr, lambda: cp_wi, lambda: cp_x(5), lambda: cp_wo, lambda: cp_hs]}
    S1_ = {2: [lambda: cp_dm, lambda: cp_ft, lambda: cp_x(4)], 4: [lambda: cp_wr, lambda: cp_wi, lambda: cp_x(5)], 6: [lambda: cp_wo, lambda: cp_hs]}
    for b in range(2, NB):
        with scope(f'w1_{b:02d}'):
            for f in W1.get(b, []): f().wait()
        for f in S1_.get(b, []): f().start(priority=1)
        if b in rng("BAR1", "-1"): bar()
        pi = proj_items(b)
        for f in mix([g for n in WORDER for g in pi[n]], plan1[b]): f()
    plan2 = {b: [] for b in range(NB)}
    add(plan2, {k[1]: v for k, v in d3.items() if k[0] == "II"})
    add(plan2, chunk([f for k in range(16) for f in st4(k)], rng("S4", "0,1,2,3,4,5,6,7")))
    add(plan2, chunk([st5(k) for k in range(16)], rng("S5", "9,10")))
    EX = {}
    for b in range(NB):
        ex = [[] for _ in range(NT_)]
        spread(plan2[b], 0, NT_, ex)
        if b > 0: spread(outproj_items(b - 1), LA + LB + HP, LA + LB + HP + E("ES", 16), ex)
        EX[b] = ex
    def marks(b):
        if b in rng("BAR2", "0"): bar()
    attn_flow(list(range(NB)), EX, marks)
    with scope('epi'):
        for f in outproj_items(NB - 1): f()
    with scope('epi_wait'):
        for b in range(NB): out_b(b).wait()
        for b in range(NB): out_a(b).wait()

_DM, _FT, _HS = a_consts2()

@jax.jit
def pallas_concat_heads__spectral_gfnet__sliding_block__prompt_kernel(A_x, A_w_r, A_w_i, B_x, B_wqkv, B_wo):
    anyspec = pl.BlockSpec(memory_space=pl.ANY)
    V = pltpu.VMEM
    return pl.pallas_call(
        kernel,
        out_shape=jax.ShapeDtypeStruct((1, S, 2*D), BF),
        in_specs=[anyspec]*9, out_specs=anyspec,
        scratch_shapes=[
            V((S, D), BF), V((DF, S), BF), V((DF, S), BF), V((16, 128, 256), BF), V((16, 256, 128), BF), V((6, 256, 256), BF),
            V((5, 16*P, 128), F32), V((6, 16, 128, 128), F32), V((6, 16, 64, 128), U32), V((2, 16, 328, 128), F32), V((S, D), BF),
            V((S, D), BF), V((D, 3*D), BF), V((D, D), BF),
            V((8, S//2, 128), U32), V((D//2, S), U32), V((D, S), F32), V((NB, D, 128), F32), V((S, D), BF),
            V((2, 5, 64, 128), U32), V((2, 128, D), BF),
            pltpu.SemaphoreType.DMA((16,)), pltpu.SemaphoreType.DMA((6,)), pltpu.SemaphoreType.DMA((7,)),
            pltpu.SemaphoreType.DMA(()), pltpu.SemaphoreType.DMA(()), pltpu.SemaphoreType.REGULAR,
        ],
        compiler_params=pltpu.CompilerParams(vmem_limit_bytes=120*2**20),
        name="kG",
    )(A_x, A_w_r.T, A_w_i.T, B_x, B_wqkv, B_wo, jnp.asarray(_FT), jnp.asarray(_HS), jnp.asarray(_DM))
```
